```python
import os as _os
_os.environ.setdefault("JAX_PLATFORMS", "cpu")
import jax
import jax.numpy as jnp

def _softmax(x, axis=-1):
    return jax.nn.softmax(x, axis=axis)
def _gelu(x):
    return jax.nn.gelu(x, approximate=True)
def _silu(x):
    return jax.nn.silu(x)
def _sigmoid(x):
    return jax.nn.sigmoid(x)
def _layernorm(x, axis=-1, eps=1e-5):
    m = jnp.mean(x, axis=axis, keepdims=True)
    v = jnp.var(x, axis=axis, keepdims=True)
    return (x - m) / jnp.sqrt(v + eps)
def _scatter_add(tgt, idx, src, axis=0):
    return tgt.at[idx].add(src)
def _segment_sum(src, seg, n):
    return jax.ops.segment_sum(src, seg, n)
class _Rng:
    def __init__(self, key):
        self._k = key
    def _next(self):
        self._k, sub = jax.random.split(self._k)
        return sub
    def normal(self, shape):
        return jax.random.normal(self._next(), shape, dtype=jnp.bfloat16)
    def randint(self, lo, hi, shape):
        return jax.random.randint(self._next(), shape, lo, hi, dtype=jnp.int32)
    def uniform(self, shape, lo=0.0, hi=1.0):
        return jax.random.uniform(self._next(), shape, jnp.bfloat16, lo, hi)
    def permutation(self, n):
        return jax.random.permutation(self._next(), n)


kernel_name = 'sequential_preLN__mha_block__moe_arch_mod__prompt'

def setup_inputs():
    _rng = _Rng(jax.random.key(int.from_bytes(__import__("os").urandom(4), "little")))
    _w = (lambda a: (lambda t: t.astype(jnp.bfloat16) if jnp.issubdtype(t.dtype, jnp.floating) else t)(jnp.asarray(a)))
    def _A_setup():
        B, S, D, H = 1, 2048, 512, 32
        return {
            "x": _w((lambda *s: _rng.normal(s) * 0.05)(B, S, D)),
            "wqkv": _w((lambda *s: _rng.normal(s) * 0.05)(D, 3 * D)),
            "wo": _w((lambda *s: _rng.normal(s) * 0.05)(D, D)),
        }
    _A_in = _A_setup()

    def _B_setup():
        B, S, D, F, C = 1, 2048, 512, 1792, 2
        return {
            "x": _w((lambda *s: _rng.normal(s) * 0.05)(B, S, D)),
            "w_r": _w((lambda *s: _rng.normal(s) * 0.05)(D)),
            "w_gate": _w((lambda *s: _rng.normal(s) * 0.05)(D, F)),
            "w_up": _w((lambda *s: _rng.normal(s) * 0.05)(D, F)),
            "w_down": _w((lambda *s: _rng.normal(s) * 0.05)(F, D)),
        }
    _B_in = _B_setup()

    return {
        "A_x": _A_in["x"],
        "A_wqkv": _A_in["wqkv"],
        "A_wo": _A_in["wo"],
        "B_x": _B_in["x"],
        "B_w_r": _B_in["w_r"],
        "B_w_gate": _B_in["w_gate"],
        "B_w_up": _B_in["w_up"],
        "B_w_down": _B_in["w_down"],
    }

def reference(A_x, A_wqkv, A_wo, B_x, B_w_r, B_w_gate, B_w_up, B_w_down):
    def _A_ref(x, wqkv, wo):
        B, S, D = x.shape
        H = 32
        Dh = D // H
        qkv = (lambda x, *d: x.transpose(*d))((x @ wqkv).reshape(B, S, 3, H, Dh), 2, 0, 3, 1, 4)
        q, k, v = qkv[0], qkv[1], qkv[2]
        scores = jnp.einsum("bhqd,bhkd->bhqk", q, k) * (Dh ** -0.5)
        p = _softmax(scores, axis=-1)
        o = jnp.einsum("bhqk,bhkd->bhqd", p, v)
        return (lambda x, *d: x.transpose(*d))(o, 0, 2, 1, 3).reshape(B, S, D) @ wo

    def _B_ref(x, w_r, w_gate, w_up, w_down):
        B, S, D = x.shape
        C = 2
        r = x @ w_r
        idx = jnp.argsort(-r, axis=-1)[:, :C]
        idx_e = jnp.repeat(idx.reshape(B, C, 1), D, axis=2)
        x_sel = jnp.take_along_axis(x, idx_e, axis=1)
        g = _silu(x_sel @ w_gate)
        u = x_sel @ w_up
        y = (g * u) @ w_down
        r_sel = _sigmoid(jnp.take_along_axis(r, idx, axis=1))
        y = y * r_sel.reshape(B, C, 1)
        b_off = (jnp.arange(B) * S).reshape(B, 1)
        flat_idx = (idx + b_off).reshape(B * C)
        zero = (x * 0.0).reshape(B * S, D)
        upd = _scatter_add(zero, flat_idx, y.reshape(B * C, D), axis=0)
        return x + upd.reshape(B, S, D)

    x = A_x
    h = x + _A_ref(_layernorm(x, axis=-1), A_wqkv, A_wo)
    h2 = h + _B_ref(_layernorm(h, axis=-1), B_w_r, B_w_gate, B_w_up, B_w_down)
    return h2
```

```python
import functools
import math

import jax
import jax.numpy as jnp
from jax import lax
import jax.experimental.pallas as pl
import jax.experimental.pallas.tpu as pltpu

f32 = jnp.float32
bf16 = jnp.bfloat16
u32 = jnp.uint32

S = 2048
D = 512
H = 32
DH = 16
F = 1792
TQ = 512
NQ = S // TQ
CK = 128
NC = S // CK
RG = 16
NR = CK // RG
DELTA = 2
OFF = 12
TB = 512
NB = S // TB
EPS = 1e-5
QSCALE = (DH ** -0.5) * math.log2(math.e)


def _ln(x):
    mu = jnp.mean(x, axis=-1, keepdims=True)
    xc = x - mu
    var = jnp.mean(xc * xc, axis=-1, keepdims=True)
    return xc * lax.rsqrt(var + EPS)


def _kernel(x_hbm, wqkv_hbm, wo_hbm, wr_hbm, wg_hbm, wu_hbm, wd_hbm, out_hbm,
            x_s, wqkv_s, wo_s, wr_s, wg_s, wu_s, wd_s,
            k_s, qt_s, vt_s, ot_s, s_s, w_s, m_s, st_s,
            hn_s, base_s, out_s, r_s, patch_s, sem_in, sem_out):
    def xcp(b):
        return pltpu.make_async_copy(x_hbm.at[pl.ds(b * TB, TB), :], x_s.at[pl.ds(b * TB, TB), :], sem_in.at[b])
    wqkv_cp = pltpu.make_async_copy(wqkv_hbm, wqkv_s, sem_in.at[NB])
    late = [pltpu.make_async_copy(src, dst, sem_in.at[NB + 1 + n])
            for n, (src, dst) in enumerate([(wo_hbm, wo_s), (wr_hbm, wr_s), (wg_hbm, wg_s), (wu_hbm, wu_s), (wd_hbm, wd_s)])]
    xcp(0).start()
    wqkv_cp.start()
    for b in range(1, NB):
        xcp(b).start()
    for cp in late:
        cp.start()

    s_s[0, (NC - DELTA) * CK:, :] = jnp.zeros((DELTA * CK, TQ), f32)
    s_s[1] = jnp.zeros((S, TQ), f32)
    m_s[...] = jnp.zeros((2, 8, TQ), f32)
    st_s[...] = jnp.ones((24, TQ), f32)

    for b in range(NB):
        xcp(b).wait()
        xn = _ln(x_s[b * TB:(b + 1) * TB, :].astype(f32)).astype(bf16)
        if b == 0:
            wqkv_cp.wait()
        k = jnp.dot(xn, wqkv_s[:, D:2 * D], preferred_element_type=f32).astype(bf16)
        for g in range(4):
            k_s[g, b * TB // 2:(b + 1) * TB // 2, :] = pltpu.bitcast(k[:, g * 128:(g + 1) * 128], u32)
        qt = (jnp.dot(xn, wqkv_s[:, 0:D], preferred_element_type=f32) * QSCALE).astype(bf16).T
        qt_s[:, b] = pltpu.bitcast(qt, u32).reshape(4, 64, TB)
        vt = jnp.dot(xn, wqkv_s[:, 2 * D:3 * D], preferred_element_type=f32).astype(bf16).T
        vt_s[:, :, b * TB:(b + 1) * TB] = pltpu.bitcast(vt, u32).reshape(H, 8, TB)

    row = lax.broadcasted_iota(jnp.int32, (64, TQ), 0) // 8

    def prep_w(h, j, slot):
        w_s[slot] = jnp.where(row == (h % 8), qt_s[h // 8, j], jnp.uint32(0))

    def a_chunk(h, slot, c, m8):
        kc = pltpu.bitcast(k_s[h // 8, c * CK // 2:(c + 1) * CK // 2, :], bf16)
        w = pltpu.bitcast(w_s[slot], bf16)
        s = jnp.dot(kc, w, preferred_element_type=f32)
        s_s[slot, c * CK:(c + 1) * CK, :] = s
        for r in range(CK // 8):
            sr = s[r * 8:(r + 1) * 8]
            m8 = sr if m8 is None else jnp.maximum(m8, sr)
        return m8, [s[r * RG:r * RG + 8] for r in range(NR)]

    def b_chunk(h, slot, c, m, l8, acc, deps, never):
        ps = []
        for r in range(NR):
            mm = m if deps[r] is None else jnp.where(never, deps[r], m)
            t = None
            for q in range(RG // 8):
                r0 = c * CK + r * RG + q * 8
                p = jnp.exp2(s_s[slot, r0:r0 + 8, :] - mm)
                ps.append(p)
                t = p if t is None else t + p
            l8 = t if l8 is None else l8 + t
        vt = pltpu.bitcast(vt_s[h, :, c * CK:(c + 1) * CK], bf16)
        pv = jnp.dot(vt, jnp.concatenate(ps, axis=0).astype(bf16), preferred_element_type=f32)
        acc = pv if acc is None else acc + pv
        return l8, acc

    def fin_b(h, j, l8, acc):
        l = l8.sum(axis=0, keepdims=True)
        ot_s[j, h] = pltpu.bitcast((acc * (1.0 / l)).astype(bf16), u32)

    def bmax(m8):
        return jnp.broadcast_to(m8.max(axis=0, keepdims=True), (8, TQ))

    prep_w(0, 0, 0)

    def body(i, carry):
        never = (lax.broadcasted_iota(jnp.int32, (8, TQ), 0) + i) < 0
        hprev = jnp.maximum(i - 1, 0)
        hnext = jnp.minimum(i + 1, H - 1)
        l8 = st_s[0:8, :]
        acc = st_s[8:24, :]
        m = bmax(m_s[0])
        mq = [m_s[1]]
        hist = []
        for t in range(NQ):
            slot = t % 2
            m8 = None
            for c in range(NC):
                rel, cb = divmod(t * NC + c - NC - DELTA, NC)
                m8, rgs = a_chunk(i, slot, c, m8)
                base = len(hist)
                hist.extend(rgs)
                if cb == 0:
                    m = bmax(mq.pop(0))
                    l8 = None
                    acc = None
                deps = [hist[base + r - OFF] if base + r - OFF >= 0 else None for r in range(NR)]
                hb = hprev if rel < 0 else i
                l8, acc = b_chunk(hb, rel % 2, cb, m, l8, acc, deps, never)
                if cb == NC - 1:
                    fin_b(hb, rel % NQ, l8, acc)
                if c == DELTA + 1:
                    if t + 1 < NQ:
                        prep_w(i, t + 1, 1 - slot)
                    else:
                        prep_w(hnext, 0, 1 - slot)
            mq.append(m8)
            if t >= NQ - 2:
                m_s[slot] = m8
        st_s[0:8, :] = l8
        st_s[8:24, :] = acc
        return carry

    lax.fori_loop(0, H, body, 0)

    none = [None] * NR
    l8 = st_s[0:8, :]
    acc = st_s[8:24, :]
    m = bmax(m_s[0])
    for cb in range(NC - DELTA, NC):
        l8, acc = b_chunk(H - 1, 0, cb, m, l8, acc, none, None)
    fin_b(H - 1, NQ - 2, l8, acc)
    m = bmax(m_s[1])
    l8 = None
    acc = None
    for cb in range(NC):
        l8, acc = b_chunk(H - 1, 1, cb, m, l8, acc, none, None)
    fin_b(H - 1, NQ - 1, l8, acc)

    for cp in late:
        cp.wait()

    def ocp(b):
        return pltpu.make_async_copy(out_s.at[pl.ds(b * TB, TB), :], out_hbm.at[pl.ds(b * TB, TB), :], sem_out.at[b])

    wr8 = jnp.broadcast_to(wr_s[...], (16, D))
    for b in range(NB):
        o = pltpu.bitcast(ot_s[b].reshape(H * 8, TQ), bf16).T
        a = jnp.dot(o, wo_s[...], preferred_element_type=f32)
        h = x_s[b * TB:(b + 1) * TB, :].astype(f32) + a
        hn = _ln(h)
        hb = hn.astype(bf16)
        base = h + hn
        hn_s[b * TB:(b + 1) * TB, :] = hn
        base_s[b * TB:(b + 1) * TB, :] = base
        out_s[b * TB:(b + 1) * TB, :] = base.astype(bf16)
        ocp(b).start()
        r = lax.dot_general(wr8, hb, (((1,), (1,)), ((), ())), preferred_element_type=f32)
        r_s[:, b * TB:(b + 1) * TB] = r[0:8]

    r = r_s[...].astype(bf16).astype(f32)
    idx = lax.broadcasted_iota(jnp.int32, (8, S), 1)
    r1 = jnp.max(r)
    i1 = jnp.min(jnp.where(r == r1, idx, S - 1))
    rm = jnp.where(idx == i1, -jnp.inf, r)
    r2 = jnp.max(rm)
    i2 = jnp.min(jnp.where((rm == r2) & (idx != i1), idx, S - 1))
    rows16 = lax.broadcasted_iota(jnp.int32, (16, D), 0)
    x1 = hn_s[pl.ds(i1, 1), :]
    x2 = hn_s[pl.ds(i2, 1), :]
    xs = jnp.where(rows16 == 0, x1, x2).astype(bf16)
    g = jnp.dot(xs, wg_s[...], preferred_element_type=f32)
    u = jnp.dot(xs, wu_s[...], preferred_element_type=f32)
    gu = (g * jax.nn.sigmoid(g) * u).astype(bf16)
    y = jnp.dot(gu, wd_s[...], preferred_element_type=f32)
    rsel = jnp.where(rows16 == 0, r1, r2)
    y = y * jax.nn.sigmoid(rsel)
    y1 = y[0:1]
    y2 = y[1:2]

    for b in range(NB):
        ocp(b).wait()
    t1 = pl.multiple_of((i1 // 16) * 16, 16)
    t2 = pl.multiple_of((i2 // 16) * 16, 16)
    for n, t in enumerate((t1, t2)):
        rid = rows16 + t
        tile = base_s[pl.ds(t, 16), :] + jnp.where(rid == i1, y1, 0.0) + jnp.where(rid == i2, y2, 0.0)
        patch_s[n] = tile.astype(bf16)
    p1 = pltpu.make_async_copy(patch_s.at[0], out_hbm.at[pl.ds(t1, 16), :], sem_out.at[NB])
    p2 = pltpu.make_async_copy(patch_s.at[1], out_hbm.at[pl.ds(t2, 16), :], sem_out.at[NB + 1])
    p1.start()

    @pl.when(t1 != t2)
    def _():
        p2.start()
        p2.wait()

    p1.wait()


@jax.jit
def pallas_sequential_preLN__mha_block__moe_arch_mod__prompt_kernel(
    A_x: jax.Array,
    A_wqkv: jax.Array,
    A_wo: jax.Array,
    B_x: jax.Array,
    B_w_r: jax.Array,
    B_w_gate: jax.Array,
    B_w_up: jax.Array,
    B_w_down: jax.Array,
):
    del B_x
    any_spec = pl.BlockSpec(memory_space=pl.ANY)
    out = pl.pallas_call(
        _kernel,
        out_shape=jax.ShapeDtypeStruct((S, D), bf16),
        in_specs=[any_spec] * 7,
        out_specs=any_spec,
        scratch_shapes=[
            pltpu.VMEM((S, D), bf16),
            pltpu.VMEM((D, 3 * D), bf16),
            pltpu.VMEM((D, D), bf16),
            pltpu.VMEM((1, D), bf16),
            pltpu.VMEM((D, F), bf16),
            pltpu.VMEM((D, F), bf16),
            pltpu.VMEM((F, D), bf16),
            pltpu.VMEM((4, S // 2, 128), u32),
            pltpu.VMEM((4, NQ, 64, TQ), u32),
            pltpu.VMEM((H, 8, S), u32),
            pltpu.VMEM((NQ, H, 8, TQ), u32),
            pltpu.VMEM((2, S, TQ), f32),
            pltpu.VMEM((2, 64, TQ), u32),
            pltpu.VMEM((2, 8, TQ), f32),
            pltpu.VMEM((24, TQ), f32),
            pltpu.VMEM((S, D), f32),
            pltpu.VMEM((S, D), f32),
            pltpu.VMEM((S, D), bf16),
            pltpu.VMEM((8, S), f32),
            pltpu.VMEM((2, 16, D), bf16),
            pltpu.SemaphoreType.DMA((NB + 6,)),
            pltpu.SemaphoreType.DMA((NB + 2,)),
        ],
        compiler_params=pltpu.CompilerParams(vmem_limit_bytes=64 * 1024 * 1024),
    )(A_x.reshape(S, D), A_wqkv, A_wo, B_w_r.reshape(1, D), B_w_gate, B_w_up, B_w_down)
    return out.reshape(1, S, D)
```

```python
import math

import jax
import jax.numpy as jnp
from jax import lax
import jax.experimental.pallas as pl
import jax.experimental.pallas.tpu as pltpu

f32 = jnp.float32
bf16 = jnp.bfloat16
u32 = jnp.uint32

S = 2048
D = 512
H = 32
DH = 16
F = 1792
TQ = 512
NQ = S // TQ
CK = 128
NC = S // CK
NV = 16
V = NV * 16
VB = -(-V // 128)
LAG = 5
VOFF = 4
HPB = 2
TB = 512
NB = S // TB
EPS = 1e-5
QSCALE = (DH ** -0.5) * math.log2(math.e)
L_LO = 2.0 ** -64
L_HI = 2.0 ** 64

_C0 = -(-V // CK)
PV_ORDER = list(range(_C0, NC)) + list(range(_C0))
_NG = (S - V) // 16
BOUNDS = [V + 16 * ((_NG * c) // NC) for c in range(NC + 1)]
PIECES = [(vg, d) for vg in range(NV) for d in range(DH)]
GENS = [(d, b) for b in range(VB) for d in range(DH)]


def _ln(x):
    mu = jnp.mean(x, axis=-1, keepdims=True)
    xc = x - mu
    var = jnp.mean(xc * xc, axis=-1, keepdims=True)
    return xc * lax.rsqrt(var + EPS)


def _kernel(x_hbm, wqkv_hbm, wo_hbm, wr_hbm, wg_hbm, wu_hbm, wd_hbm, out_hbm,
            x_s, wqkv_s, wo_s, wg_s, wu_s, wd_s,
            k_s, qt_s, vt_s, ot_s, kt_s, kb0_s, kb1_s, qb_s, p_s, w_s, l_s, st_s, bad_s,
            hn_s, base_s, out_s, r_s, patch_s, wr_s, sem_in, sem_out):
    def xcp(b):
        return pltpu.make_async_copy(x_hbm.at[pl.ds(b * TB, TB), :], x_s.at[pl.ds(b * TB, TB), :], sem_in.at[b])

    def wcp(n):
        return pltpu.make_async_copy(wqkv_hbm.at[:, pl.ds(n * D, D)], wqkv_s.at[n], sem_in.at[NB + n])

    late = [pltpu.make_async_copy(src, dst, sem_in.at[NB + 3 + n])
            for n, (src, dst) in enumerate([(wo_hbm, wo_s), (wr_hbm, wr_s), (wg_hbm, wg_s), (wu_hbm, wu_s), (wd_hbm, wd_s)])]
    xcp(0).start()
    wcp(1).start()
    xcp(1).start()
    wcp(0).start()
    wcp(2).start()
    for b in range(2, NB):
        xcp(b).start()

    for k in range(NC - LAG, NC):
        c = PV_ORDER[k]
        p_s[1, c * CK:(c + 1) * CK, :] = jnp.zeros((CK, TQ), bf16)
    l_s[...] = jnp.ones((8, TQ), f32)
    st_s[...] = jnp.ones((DH, TQ), f32)
    bad_s[...] = jnp.zeros((8, TQ), f32)

    kbs = [kb0_s, kb1_s]
    row = lax.broadcasted_iota(jnp.int32, (64, TQ), 0) // 8

    def head_weights(h, j):
        return jnp.where(row == (h % 8), qt_s[h // 8, j], jnp.uint32(0))

    def prep_w(h, j, slot):
        w_s[slot] = head_weights(h, j)
        q16 = pltpu.bitcast(qt_s[h // 8, j, pl.ds(pl.multiple_of((h % 8) * 8, 8), 8), :], bf16).astype(f32)
        for d in range(DH):
            qb_s[slot, d * 8:(d + 1) * 8, :] = jnp.broadcast_to(q16[d:d + 1], (8, TQ))

    def gen_kb(h, kb, d, b):
        rowv = kt_s[h, d:d + 1, b * 128:(b + 1) * 128]
        kb[d, b * 128:(b + 1) * 128, :] = jnp.broadcast_to(rowv, (128, 128)).T

    def ln1(b):
        return _ln(x_s[b * TB:(b + 1) * TB, :].astype(f32)).astype(bf16)

    def proj_k(b, xn):
        k = jnp.dot(xn, wqkv_s[1], preferred_element_type=f32).astype(bf16)
        for g in range(4):
            k_s[g, b * TB // 2:(b + 1) * TB // 2, :] = pltpu.bitcast(k[:, g * 128:(g + 1) * 128], u32)
        if b == 0:
            kt_s[...] = k[0:VB * 128].T.astype(f32).reshape(H, DH, VB * 128)

    def proj_q(b, xn):
        qt = (jnp.dot(xn, wqkv_s[0], preferred_element_type=f32) * QSCALE).astype(bf16).T
        qt_s[:, b] = pltpu.bitcast(qt, u32).reshape(4, 64, TB)

    def proj_v(b, xn):
        vt = jnp.dot(xn, wqkv_s[2], preferred_element_type=f32).astype(bf16).T
        vt_s[:, :, b * TB:(b + 1) * TB] = pltpu.bitcast(vt, u32).reshape(H, 8, TB)

    xcp(0).wait()
    xn0 = ln1(0)
    wcp(1).wait()
    proj_k(0, xn0)
    xcp(1).wait()
    wcp(0).wait()
    proj_q(0, xn0)
    xn1 = ln1(1)
    proj_k(1, xn1)
    wcp(2).wait()
    for b in range(2, NB):
        xcp(b).wait()
    for cp in late:
        cp.start()
    proj_v(0, xn0)
    for d, b in GENS:
        gen_kb(0, kb0_s, d, b)
    prep_w(0, 0, 0)
    proj_q(1, xn1)
    proj_v(1, xn1)
    for b in range(2, NB):
        xn = ln1(b)
        proj_k(b, xn)
        proj_q(b, xn)
        proj_v(b, xn)
    for cp in late:
        cp.wait()

    def finish_rows(slot, r0, s, l8):
        p = jnp.exp2(s)
        for r in range(0, s.shape[0], 16):
            t = p[r:r + 8] + p[r + 8:r + 16]
            l8 = t if l8 is None else l8 + t
        p_s[slot, r0:r0 + s.shape[0], :] = p.astype(bf16)
        return l8

    def pv_chunk(h, slot, c, acc):
        vt = pltpu.bitcast(vt_s[h, :, c * CK:(c + 1) * CK], bf16)
        pv = jnp.dot(vt, p_s[slot, c * CK:(c + 1) * CK, :], preferred_element_type=f32)
        return pv if acc is None else acc + pv

    def fin(h, j, l8, acc):
        l = l8.sum(axis=0, keepdims=True)
        o = acc * (1.0 / l)
        ot_s[j, h] = pltpu.bitcast(o.astype(bf16), u32)
        oo = jnp.maximum(jnp.abs(o[0:8]), jnp.abs(o[8:16]))
        good = (l >= L_LO) & (l <= L_HI) & (oo <= 3e38)
        bad_s[...] = jnp.where(good, bad_s[...], 1.0)

    def body(i, carry):
        zero = jnp.minimum(i, 0)
        never = (lax.broadcasted_iota(jnp.int32, (16, 128), 0) + i) < 0
        acc = st_s[...]
        lq = [l_s[...]]
        hist = []
        for hh in range(HPB):
            h = i * HPB + hh
            hprev = jnp.maximum(h - 1, 0) if hh == 0 else h - 1
            hnext = jnp.minimum(h + 1, H - 1) if hh == HPB - 1 else h + 1
            kbr = kbs[hh % 2]
            for t in range(NQ):
                slot = t % 2
                l8 = None
                l8v = None
                vacc = None
                for c in range(NC):
                    r0, r1 = BOUNDS[c], BOUNDS[c + 1]
                    kc = pltpu.bitcast(k_s[h // 8, r0 // 2:r1 // 2, :], bf16)
                    s = jnp.dot(kc, pltpu.bitcast(w_s[slot], bf16), preferred_element_type=f32)
                    base = len(hist)
                    hist.extend([s[r:r + 8, 0:128] for r in range(0, r1 - r0, 8)])
                    n_new = len(hist) - base
                    l8 = finish_rows(slot, r0, s, l8)
                    pcs = PIECES[(len(PIECES) * c) // NC:(len(PIECES) * (c + 1)) // NC]
                    for n, (vg, d) in enumerate(pcs):
                        kb = kbr[zero + d, vg * 16:(vg + 1) * 16, :]
                        ii = base + (n * n_new) // len(pcs) - VOFF
                        if ii >= 0:
                            kb = jnp.where(never, jnp.concatenate([hist[ii]] * 2, axis=0), kb)
                        qb8 = qb_s[slot, d * 8:(d + 1) * 8, :]
                        tt = jnp.concatenate([kb] * 4, axis=1) * jnp.concatenate([qb8] * 2, axis=0)
                        vacc = tt if d == 0 else vacc + tt
                        if d == DH - 1:
                            l8v = finish_rows(slot, vg * 16, vacc, l8v)
                    rel, k = divmod(t * NC + c - LAG, NC)
                    hb = hprev if rel < 0 else h
                    if k == 0:
                        acc = None
                    acc = pv_chunk(hb, rel % 2, PV_ORDER[k], acc)
                    if k == NC - 1:
                        fin(hb, rel % NQ, lq.pop(0), acc)
                    if c == LAG:
                        if t + 1 < NQ:
                            prep_w(h, t + 1, 1 - slot)
                        else:
                            prep_w(hnext, 0, 1 - slot)
                    st = t * NC + c
                    for gi in range((len(GENS) * st) // (NQ * NC), (len(GENS) * (st + 1)) // (NQ * NC)):
                        gen_kb(hnext, kbs[(hh + 1) % 2], *GENS[gi])
                lq.append(l8 + l8v)
        st_s[...] = acc
        l_s[...] = lq[0]
        return carry

    lax.fori_loop(0, H // HPB, body, 0)

    acc = st_s[...]
    for k in range(NC - LAG, NC):
        acc = pv_chunk(H - 1, 1, PV_ORDER[k], acc)
    fin(H - 1, NQ - 1, l_s[...], acc)

    @pl.when(jnp.max(bad_s[...]) > 0.0)
    def _():
        def unit(u, carry):
            h = u // NQ
            j = u % NQ
            w_s[0] = head_weights(h, j)

            def scores(c, m8):
                r = pl.multiple_of(c * 128, 128)
                kc = pltpu.bitcast(k_s[h // 8, pl.ds(pl.multiple_of(c * 64, 64), 64), :], bf16)
                s = jnp.dot(kc, pltpu.bitcast(w_s[0], bf16), preferred_element_type=f32)
                hn_s[pl.ds(r, 128), :] = s
                return jnp.maximum(m8, s.reshape(16, 8, TQ).max(axis=0))

            m8 = lax.fori_loop(0, NC, scores, jnp.full((8, TQ), -jnp.inf, f32))
            m = m8.max(axis=0, keepdims=True)

            def probs(c, l8):
                r = pl.multiple_of(c * 128, 128)
                p = jnp.exp2(hn_s[pl.ds(r, 128), :] - m)
                p_s[0, pl.ds(r, 128), :] = p.astype(bf16)
                return l8 + p.reshape(16, 8, TQ).sum(axis=0)

            l8 = lax.fori_loop(0, NC, probs, jnp.zeros((8, TQ), f32))
            vt = pltpu.bitcast(vt_s[h], bf16)
            o = jnp.dot(vt, p_s[0], preferred_element_type=f32) * (1.0 / l8.sum(axis=0, keepdims=True))
            ot_s[j, h] = pltpu.bitcast(o.astype(bf16), u32)
            return carry

        lax.fori_loop(0, H * NQ, unit, 0)

    def ocp(b):
        return pltpu.make_async_copy(out_s.at[pl.ds(b * TB, TB), :], out_hbm.at[pl.ds(b * TB, TB), :], sem_out.at[b])

    wr16 = wr_s[...]

    def oproj(b, lo, n):
        o = pltpu.bitcast(ot_s[b, :, :, lo:lo + n].reshape(H * 8, n), bf16).T
        return jnp.dot(o, wo_s[...], preferred_element_type=f32)

    def post(r0, a):
        n = a.shape[0]
        h = x_s[r0:r0 + n, :].astype(f32) + a
        hn = _ln(h)
        base = h + hn
        hn_s[r0:r0 + n, :] = hn
        base_s[r0:r0 + n, :] = base
        out_s[r0:r0 + n, :] = base.astype(bf16)
        r = lax.dot_general(wr16, hn.astype(bf16), (((1,), (1,)), ((), ())), preferred_element_type=f32)
        r_s[:, r0:r0 + n] = r[0:8]

    for b in range(NB - 1):
        post(b * TB, oproj(b, 0, TB))
    hb2 = TB // 2
    post((NB - 1) * TB, oproj(NB - 1, 0, hb2))
    a_last = oproj(NB - 1, hb2, hb2)
    for b in range(NB - 1):
        ocp(b).start()
    post((NB - 1) * TB + hb2, a_last)
    ocp(NB - 1).start()

    r = r_s[...].astype(bf16).astype(f32)
    idx = lax.broadcasted_iota(jnp.int32, (8, S), 1)
    r1 = jnp.max(r)
    i1 = jnp.min(jnp.where(r == r1, idx, S - 1))
    rm = jnp.where(idx == i1, -jnp.inf, r)
    r2 = jnp.max(rm)
    i2 = jnp.min(jnp.where((rm == r2) & (idx != i1), idx, S - 1))
    rows16 = lax.broadcasted_iota(jnp.int32, (16, D), 0)
    x1 = hn_s[pl.ds(i1, 1), :]
    x2 = hn_s[pl.ds(i2, 1), :]
    xs = jnp.where(rows16 == 0, x1, x2).astype(bf16)
    g = jnp.dot(xs, wg_s[...], preferred_element_type=f32)
    u = jnp.dot(xs, wu_s[...], preferred_element_type=f32)
    gu = (g * jax.nn.sigmoid(g) * u).astype(bf16)
    y = jnp.dot(gu, wd_s[...], preferred_element_type=f32)
    rsel = jnp.where(rows16 == 0, r1, r2)
    y = y * jax.nn.sigmoid(rsel)
    y1 = y[0:1]
    y2 = y[1:2]

    t1 = pl.multiple_of((i1 // 16) * 16, 16)
    t2 = pl.multiple_of((i2 // 16) * 16, 16)
    for n, t in enumerate((t1, t2)):
        rid = rows16 + t
        tile = base_s[pl.ds(t, 16), :] + jnp.where(rid == i1, y1, 0.0) + jnp.where(rid == i2, y2, 0.0)
        patch_s[n] = tile.astype(bf16)
    for b in range(NB):
        ocp(b).wait()
    p1 = pltpu.make_async_copy(patch_s.at[0], out_hbm.at[pl.ds(t1, 16), :], sem_out.at[NB])
    p2 = pltpu.make_async_copy(patch_s.at[1], out_hbm.at[pl.ds(t2, 16), :], sem_out.at[NB + 1])
    p1.start()

    @pl.when(t1 != t2)
    def _():
        p2.start()
        p2.wait()

    p1.wait()


@jax.jit
def pallas_sequential_preLN__mha_block__moe_arch_mod__prompt_kernel(
    A_x: jax.Array,
    A_wqkv: jax.Array,
    A_wo: jax.Array,
    B_x: jax.Array,
    B_w_r: jax.Array,
    B_w_gate: jax.Array,
    B_w_up: jax.Array,
    B_w_down: jax.Array,
):
    del B_x
    any_spec = pl.BlockSpec(memory_space=pl.ANY)
    out = pl.pallas_call(
        _kernel,
        out_shape=jax.ShapeDtypeStruct((S, D), bf16),
        in_specs=[any_spec] * 7,
        out_specs=any_spec,
        scratch_shapes=[
            pltpu.VMEM((S, D), bf16),
            pltpu.VMEM((3, D, D), bf16),
            pltpu.VMEM((D, D), bf16),
            pltpu.VMEM((D, F), bf16),
            pltpu.VMEM((D, F), bf16),
            pltpu.VMEM((F, D), bf16),
            pltpu.VMEM((4, S // 2, 128), u32),
            pltpu.VMEM((4, NQ, 64, TQ), u32),
            pltpu.VMEM((H, 8, S), u32),
            pltpu.VMEM((NQ, H, 8, TQ), u32),
            pltpu.VMEM((H, DH, VB * 128), f32),
            pltpu.VMEM((DH, VB * 128, 128), f32),
            pltpu.VMEM((DH, VB * 128, 128), f32),
            pltpu.VMEM((2, DH * 8, TQ), f32),
            pltpu.VMEM((2, S, TQ), bf16),
            pltpu.VMEM((2, 64, TQ), u32),
            pltpu.VMEM((8, TQ), f32),
            pltpu.VMEM((DH, TQ), f32),
            pltpu.VMEM((8, TQ), f32),
            pltpu.VMEM((S, D), f32),
            pltpu.VMEM((S, D), f32),
            pltpu.VMEM((S, D), bf16),
            pltpu.VMEM((8, S), f32),
            pltpu.VMEM((2, 16, D), bf16),
            pltpu.VMEM((16, D), bf16),
            pltpu.SemaphoreType.DMA((NB + 8,)),
            pltpu.SemaphoreType.DMA((NB + 2,)),
        ],
        compiler_params=pltpu.CompilerParams(vmem_limit_bytes=80 * 1024 * 1024),
    )(A_x.reshape(S, D), A_wqkv, A_wo, jnp.broadcast_to(B_w_r[None, :], (16, D)), B_w_gate, B_w_up, B_w_down)
    return out.reshape(1, S, D)
```

```python
import math

import jax
import jax.numpy as jnp
from jax import lax
import jax.experimental.pallas as pl
import jax.experimental.pallas.tpu as pltpu

f32 = jnp.float32
bf16 = jnp.bfloat16
u32 = jnp.uint32

S = 2048
D = 512
H = 32
DH = 16
F = 1792
TQ = 512
NQ = S // TQ
CK = 128
NC = S // CK
NV = 16
V = NV * 16
VB = -(-V // 128)
LAG = 4
VOFF = 4
HPB = 2
TB = 512
NB = S // TB
EB = 512
LB = 32
EPS = 1e-5
QSCALE = (DH ** -0.5) * math.log2(math.e)
L_LO = 2.0 ** -64
L_HI = 2.0 ** 64

_C0 = -(-V // CK)
PV_ORDER = list(range(_C0, NC)) + list(range(_C0))
_NG = (S - V) // 16
BOUNDS = [V + 16 * ((_NG * c) // NC) for c in range(NC + 1)]
PIECES = [(vg, d) for vg in range(NV) for d in range(DH)]
GENS = [(d, b) for b in range(VB) for d in range(DH)]


def _ln(x):
    mu = jnp.mean(x, axis=-1, keepdims=True)
    xc = x - mu
    var = jnp.mean(xc * xc, axis=-1, keepdims=True)
    return xc * lax.rsqrt(var + EPS)


def _kernel(x_hbm, wqkv_hbm, wo_hbm, wr_hbm, wg_hbm, wu_hbm, wd_hbm, out_hbm,
            x_s, wqkv_s, wo_s, wg_s, wu_s, wd_s,
            k_s, qt_s, vt_s, ot_s, kt_s, kb0_s, kb1_s, qb_s, p_s, w_s, l_s, st_s, bad_s,
            hn_s, s_s, out_s, r_s, patch_s, wr_s, sem_in, sem_out):
    def xcp(b):
        return pltpu.make_async_copy(x_hbm.at[pl.ds(b * TB, TB), :], x_s.at[pl.ds(b * TB, TB), :], sem_in.at[b])

    def wcp(n):
        return pltpu.make_async_copy(wqkv_hbm.at[:, pl.ds(n * D, D)], wqkv_s.at[n], sem_in.at[NB + n])

    late = [pltpu.make_async_copy(src, dst, sem_in.at[NB + 3 + n])
            for n, (src, dst) in enumerate([(wo_hbm, wo_s), (wr_hbm, wr_s.at[pl.ds(0, D)]), (wg_hbm, wg_s), (wu_hbm, wu_s), (wd_hbm, wd_s)])]
    xcp(0).start()
    wcp(1).start()
    xcp(1).start()
    wcp(0).start()
    wcp(2).start()
    for b in range(2, NB):
        xcp(b).start()

    for k in range(NC - LAG, NC):
        c = PV_ORDER[k]
        p_s[(S + c * CK) // 2:(S + (c + 1) * CK) // 2, :] = jnp.zeros((CK // 2, TQ), u32)
    l_s[...] = jnp.ones((8, TQ), f32)
    st_s[...] = jnp.ones((DH, TQ), f32)
    bad_s[...] = jnp.zeros((8, TQ), f32)

    kbs = [kb0_s, kb1_s]
    row = lax.broadcasted_iota(jnp.int32, (64, TQ), 0) // 8

    def head_weights(h, j):
        return jnp.where(row == (h % 8), qt_s[h // 8, j], jnp.uint32(0))

    def prep_w(h, j, slot):
        w_s[slot] = head_weights(h, j)
        q16 = pltpu.bitcast(qt_s[h // 8, j, pl.ds(pl.multiple_of((h % 8) * 8, 8), 8), :], bf16).astype(f32)
        for d in range(DH):
            qb_s[slot, d * 8:(d + 1) * 8, :] = jnp.broadcast_to(q16[d:d + 1], (8, TQ))

    def gen_kb(h, kb, d, b):
        rowv = kt_s[h, d:d + 1, b * 128:(b + 1) * 128]
        kb[d, b * 128:(b + 1) * 128, :] = jnp.broadcast_to(rowv, (128, 128)).T

    def ln1(b):
        return _ln(x_s[b * TB:(b + 1) * TB, :].astype(f32)).astype(bf16)

    def proj_k(b, xn):
        k = jnp.dot(xn, wqkv_s[1], preferred_element_type=f32).astype(bf16)
        for g in range(4):
            k_s.at[g][b * TB // 2:(b + 1) * TB // 2, :] = pltpu.bitcast(k[:, g * 128:(g + 1) * 128], u32)
        if b == 0:
            kt_s[...] = k[0:VB * 128].T.astype(f32).reshape(H, DH, VB * 128)

    def proj_q(b, xn):
        qt = (jnp.dot(xn, wqkv_s[0], preferred_element_type=f32) * QSCALE).astype(bf16).T
        qt_s[:, b] = pltpu.bitcast(qt, u32).reshape(4, 64, TB)

    def proj_v(b, xn):
        vt = jnp.dot(xn, wqkv_s[2], preferred_element_type=f32).astype(bf16).T
        vt_s[:, :, b * TB:(b + 1) * TB] = pltpu.bitcast(vt, u32).reshape(H, 8, TB)

    xcp(0).wait()
    xn0 = ln1(0)
    wcp(1).wait()
    proj_k(0, xn0)
    xcp(1).wait()
    wcp(0).wait()
    proj_q(0, xn0)
    xn1 = ln1(1)
    proj_k(1, xn1)
    wcp(2).wait()
    for b in range(2, NB):
        xcp(b).wait()
    for cp in late:
        cp.start()
    proj_v(0, xn0)
    for d, b in GENS:
        gen_kb(0, kb0_s, d, b)
    prep_w(0, 0, 0)
    proj_q(1, xn1)
    proj_v(1, xn1)
    for b in range(2, NB):
        xn = ln1(b)
        proj_k(b, xn)
        proj_q(b, xn)
        proj_v(b, xn)
    for cp in late:
        cp.wait()

    def finish_rows(slot, r0, s, l8):
        p = jnp.exp2(s)
        for r in range(0, s.shape[0], 16):
            t = p[r:r + 8] + p[r + 8:r + 16]
            l8 = t if l8 is None else l8 + t
        r0 = slot * S + r0
        p_s[r0 // 2:(r0 + s.shape[0]) // 2, :] = pltpu.bitcast(p.astype(bf16), u32)
        return l8

    def pv_chunk(h, slot, c, acc):
        vt = pltpu.bitcast(vt_s[h, :, c * CK:(c + 1) * CK], bf16)
        r0 = slot * S + c * CK
        pv = jnp.dot(vt, pltpu.bitcast(p_s[r0 // 2:(r0 + CK) // 2, :], bf16), preferred_element_type=f32)
        return pv if acc is None else acc + pv

    def fin(h, j, l8, acc):
        l = l8.sum(axis=0, keepdims=True)
        o = acc * (1.0 / l)
        ot_s.at[j, h][...] = pltpu.bitcast(o.astype(bf16), u32)
        oo = jnp.maximum(jnp.abs(o[0:8]), jnp.abs(o[8:16]))
        good = (l >= L_LO) & (l <= L_HI) & (oo <= 3e38)
        bad_s[...] = jnp.where(good, bad_s[...], 1.0)

    def body(i, carry):
        zero = jnp.minimum(i, 0)
        never = (lax.broadcasted_iota(jnp.int32, (16, 128), 0) + i) < 0
        lq = [l_s[...]]
        hist = []
        for hh in range(HPB):
            h = i * HPB + hh
            hprev = jnp.maximum(h - 1, 0) if hh == 0 else h - 1
            hnext = jnp.minimum(h + 1, H - 1) if hh == HPB - 1 else h + 1
            kbr = kbs[hh % 2]
            for t in range(NQ):
                slot = t % 2
                l8 = None
                l8v = None
                vacc = None
                for c in range(NC):
                    r0, r1 = BOUNDS[c], BOUNDS[c + 1]
                    kc = pltpu.bitcast(k_s[h // 8, r0 // 2:r1 // 2, :], bf16)
                    s = jnp.dot(kc, pltpu.bitcast(w_s[slot], bf16), preferred_element_type=f32)
                    base = len(hist)
                    hist.extend([s[r:r + 8, 0:128] for r in range(0, r1 - r0, 8)])
                    n_new = len(hist) - base
                    l8 = finish_rows(slot, r0, s, l8)
                    pcs = PIECES[(len(PIECES) * c) // NC:(len(PIECES) * (c + 1)) // NC]
                    for n, (vg, d) in enumerate(pcs):
                        kb = kbr[zero + d, vg * 16:(vg + 1) * 16, :]
                        ii = base + (n * n_new) // len(pcs) - VOFF
                        if ii >= 0:
                            kb = jnp.where(never, jnp.concatenate([hist[ii]] * 2, axis=0), kb)
                        qb8 = qb_s[slot, d * 8:(d + 1) * 8, :]
                        tt = jnp.concatenate([kb] * 4, axis=1) * jnp.concatenate([qb8] * 2, axis=0)
                        vacc = tt if d == 0 else vacc + tt
                        if d == DH - 1:
                            l8v = finish_rows(slot, vg * 16, vacc, l8v)
                    rel, k = divmod(t * NC + c - LAG, NC)
                    hb = hprev if rel < 0 else h
                    acc = pv_chunk(hb, rel % 2, PV_ORDER[k], None if k == 0 else st_s[...])
                    if k == NC - 1:
                        fin(hb, rel % NQ, lq.pop(0), acc)
                    else:
                        st_s[...] = acc
                    if c == LAG:
                        if t + 1 < NQ:
                            prep_w(h, t + 1, 1 - slot)
                        else:
                            prep_w(hnext, 0, 1 - slot)
                    st = t * NC + c
                    for gi in range((len(GENS) * st) // (NQ * NC), (len(GENS) * (st + 1)) // (NQ * NC)):
                        gen_kb(hnext, kbs[(hh + 1) % 2], *GENS[gi])
                lq.append(l8 + l8v)
        l_s[...] = lq[0]
        return carry

    lax.fori_loop(0, H // HPB, body, 0)

    acc = st_s[...]
    for k in range(NC - LAG, NC):
        acc = pv_chunk(H - 1, 1, PV_ORDER[k], acc)
    fin(H - 1, NQ - 1, l_s[...], acc)

    @pl.when(jnp.max(bad_s[...]) > 0.0)
    def _():
        def unit(u, carry):
            h = u // NQ
            j = u % NQ
            w_s[0] = head_weights(h, j)

            def scores(c, m8):
                r = pl.multiple_of(c * 128, 128)
                kc = pltpu.bitcast(k_s[h // 8, pl.ds(pl.multiple_of(c * 64, 64), 64), :], bf16)
                s = jnp.dot(kc, pltpu.bitcast(w_s[0], bf16), preferred_element_type=f32)
                s_s[pl.ds(r, 128), :] = s
                return jnp.maximum(m8, s.reshape(16, 8, TQ).max(axis=0))

            m8 = lax.fori_loop(0, NC, scores, jnp.full((8, TQ), -jnp.inf, f32))
            m = m8.max(axis=0, keepdims=True)

            def probs(c, l8):
                r = pl.multiple_of(c * 128, 128)
                p = jnp.exp2(s_s[pl.ds(r, 128), :] - m)
                p_s[pl.ds(pl.multiple_of(c * 64, 64), 64), :] = pltpu.bitcast(p.astype(bf16), u32)
                return l8 + p.reshape(16, 8, TQ).sum(axis=0)

            l8 = lax.fori_loop(0, NC, probs, jnp.zeros((8, TQ), f32))
            vt = pltpu.bitcast(vt_s[h], bf16)
            o = jnp.dot(vt, pltpu.bitcast(p_s[0:S // 2, :], bf16), preferred_element_type=f32) * (1.0 / l8.sum(axis=0, keepdims=True))
            ot_s[j, h] = pltpu.bitcast(o.astype(bf16), u32)
            return carry

        lax.fori_loop(0, H * NQ, unit, 0)

    def ocp(b):
        return pltpu.make_async_copy(out_s.at[pl.ds(b * TB, TB), :], out_hbm.at[pl.ds(b * TB, TB), :], sem_out.at[b])

    w4 = wr_s[0:D].reshape(4, 128).astype(f32)
    wr16 = jnp.concatenate([jnp.broadcast_to(w4[j:j + 1], (16, 128)) for j in range(4)], axis=1).astype(bf16)

    def oproj(b, lo, n):
        o = pltpu.bitcast(ot_s[b, :, :, lo:lo + n].reshape(H * 8, n), bf16).T
        return jnp.dot(o, wo_s[...], preferred_element_type=f32)

    def post(r0, a):
        n = a.shape[0]
        hbs = []
        for q in range(0, n, LB):
            h = x_s[r0 + q:r0 + q + LB, :].astype(f32) + a[q:q + LB]
            hn = _ln(h)
            out_s[r0 + q:r0 + q + LB, :] = (h + hn).astype(bf16)
            hn_s[(r0 + q) // 2:(r0 + q + LB) // 2, :] = pltpu.bitcast(hn.astype(bf16), u32)
        hb = pltpu.bitcast(hn_s[r0 // 2:(r0 + n) // 2, :], bf16)
        r = lax.dot_general(wr16, hb, (((1,), (1,)), ((), ())), preferred_element_type=f32)
        r_s[:, r0:r0 + n] = r[0:8]

    subs = [(b, lo) for b in range(NB) for lo in range(0, TB, EB)]
    a_next = oproj(0, 0, EB)
    for n, (b, lo) in enumerate(subs):
        a_cur = a_next
        if n + 1 < len(subs):
            a_next = oproj(subs[n + 1][0], subs[n + 1][1], EB)
        if n == len(subs) - 1:
            for bb in range(NB - 1):
                ocp(bb).start()
        post(b * TB + lo, a_cur)
    ocp(NB - 1).start()

    bits = pltpu.bitcast(r_s[...].astype(bf16).astype(f32), jnp.int32)
    idx = lax.broadcasted_iota(jnp.int32, (8, S), 1)
    key = ((bits ^ ((bits >> 31) & 0x7FFFFFFF)) & -65536) | (S - 1 - idx)
    k1 = jnp.max(key, axis=1, keepdims=True)
    k2 = jnp.max(jnp.where(key == k1, jnp.iinfo(jnp.int32).min, key), axis=1, keepdims=True)
    i1 = S - 1 - (k1[0, 0] & 0xFFFF)
    i2 = S - 1 - (k2[0, 0] & 0xFFFF)

    def key_score(k):
        hi = k & -65536
        return pltpu.bitcast(jnp.broadcast_to((hi ^ ((hi >> 31) & 0x7FFFFFFF)) & -65536, (8, 128)), f32)[0:1, 0:1]

    r1 = key_score(k1)
    r2 = key_score(k2)
    rows16 = lax.broadcasted_iota(jnp.int32, (16, D), 0)
    t1 = pl.multiple_of((i1 // 16) * 16, 16)
    t2 = pl.multiple_of((i2 // 16) * 16, 16)
    xs = pltpu.bitcast(jnp.concatenate([hn_s[pl.ds(pl.multiple_of(t // 2, 8), 8), :] for t in (t1, t2)], axis=0), bf16)
    g = jnp.dot(xs, wg_s[...], preferred_element_type=f32)
    u = jnp.dot(xs, wu_s[...], preferred_element_type=f32)
    gu = (g * jax.nn.sigmoid(g) * u).astype(bf16)
    y = jnp.dot(gu, wd_s[...], preferred_element_type=f32)
    s1 = jax.nn.sigmoid(r1)
    s2 = jax.nn.sigmoid(r2)
    for n, t in enumerate((t1, t2)):
        rid = rows16 + t
        yt = y[n * 16:(n + 1) * 16]
        upd = jnp.where(rid == i1, yt * s1, jnp.where(rid == i2, yt * s2, 0.0))
        patch_s[n] = (out_s[pl.ds(t, 16), :].astype(f32) + upd).astype(bf16)
    for b in range(NB):
        ocp(b).wait()
    p1 = pltpu.make_async_copy(patch_s.at[0], out_hbm.at[pl.ds(t1, 16), :], sem_out.at[NB])
    p2 = pltpu.make_async_copy(patch_s.at[1], out_hbm.at[pl.ds(t2, 16), :], sem_out.at[NB + 1])
    p1.start()

    @pl.when(t1 != t2)
    def _():
        p2.start()
        p2.wait()

    p1.wait()


@jax.jit
def pallas_sequential_preLN__mha_block__moe_arch_mod__prompt_kernel(
    A_x: jax.Array,
    A_wqkv: jax.Array,
    A_wo: jax.Array,
    B_x: jax.Array,
    B_w_r: jax.Array,
    B_w_gate: jax.Array,
    B_w_up: jax.Array,
    B_w_down: jax.Array,
):
    del B_x
    any_spec = pl.BlockSpec(memory_space=pl.ANY)
    out = pl.pallas_call(
        _kernel,
        out_shape=jax.ShapeDtypeStruct((S, D), bf16),
        in_specs=[any_spec] * 7,
        out_specs=any_spec,
        scratch_shapes=[
            pltpu.VMEM((S, D), bf16),
            pltpu.VMEM((3, D, D), bf16),
            pltpu.VMEM((D, D), bf16),
            pltpu.VMEM((D, F), bf16),
            pltpu.VMEM((D, F), bf16),
            pltpu.VMEM((F, D), bf16),
            pltpu.VMEM((4, S // 2, 128), u32),
            pltpu.VMEM((4, NQ, 64, TQ), u32),
            pltpu.VMEM((H, 8, S), u32),
            pltpu.VMEM((NQ, H, 8, TQ), u32),
            pltpu.VMEM((H, DH, VB * 128), f32),
            pltpu.VMEM((DH, VB * 128, 128), f32),
            pltpu.VMEM((DH, VB * 128, 128), f32),
            pltpu.VMEM((2, DH * 8, TQ), f32),
            pltpu.VMEM((S, TQ), u32),
            pltpu.VMEM((2, 64, TQ), u32),
            pltpu.VMEM((8, TQ), f32),
            pltpu.VMEM((DH, TQ), f32),
            pltpu.VMEM((8, TQ), f32),
            pltpu.VMEM((S // 2, D), u32),
            pltpu.VMEM((S, TQ), f32),
            pltpu.VMEM((S, D), bf16),
            pltpu.VMEM((8, S), f32),
            pltpu.VMEM((2, 16, D), bf16),
            pltpu.VMEM((4 * D,), bf16),
            pltpu.SemaphoreType.DMA((NB + 8,)),
            pltpu.SemaphoreType.DMA((NB + 2,)),
        ],
        compiler_params=pltpu.CompilerParams(vmem_limit_bytes=80 * 1024 * 1024),
    )(A_x.reshape(S, D), A_wqkv, A_wo, B_w_r, B_w_gate, B_w_up, B_w_down)
    return out.reshape(1, S, D)
```

```python
import math

import jax
import jax.numpy as jnp
from jax import lax
import jax.experimental.pallas as pl
import jax.experimental.pallas.tpu as pltpu

f32 = jnp.float32
bf16 = jnp.bfloat16
u32 = jnp.uint32

S = 2048
D = 512
H = 32
DH = 16
F = 1792
TQ = 512
NQ = S // TQ
CK = 128
NC = S // CK
NV = 16
V = NV * 16
VB = V // 128
LAG = 4
VOFF = 4
HPB = 2
EB = 256
OUT_STARTS = (4, 7)
EPS = 1e-5
QSCALE = (DH ** -0.5) * math.log2(math.e)
L_LO = 2.0 ** -64
L_HI = 2.0 ** 64
V_HI = 2.0 ** 60

PV_ORDER = list(range(VB, NC)) + list(range(VB))
BOUNDS = [V + 16 * ((((S - V) // 16) * c) // NC) for c in range(NC + 1)]
PIECES = [(vg, d) for vg in range(NV) for d in range(DH)]
GENS = [(d, b) for b in range(VB) for d in range(DH)]


def _ln(x):
    mu = jnp.mean(x, axis=-1, keepdims=True)
    xc = x - mu
    var = jnp.mean(xc * xc, axis=-1, keepdims=True)
    return xc * lax.rsqrt(var + EPS)


def _pack(x):
    return pltpu.bitcast(x.astype(bf16), u32)


def _unpack(x):
    return pltpu.bitcast(x, bf16)


def _kernel(x_hbm, wqkv_hbm, wo_hbm, wr_hbm, wg_hbm, wu_hbm, wd_hbm, out_hbm,
            x_s, wqkv_s, wo_s, wg_s, wu_s, wd_s,
            k_s, qt_s, vt_s, ot_s, kt_s, kbe_s, kbo_s, qf_s, p_s, w0_s, w1_s, l_s, acc_s, bad_s,
            hn_s, s_s, out_s, r_s, patch_s, wr_s, sem_in, sem_out):
    def xcp(b):
        return pltpu.make_async_copy(x_hbm.at[pl.ds(b * TQ, TQ), :], x_s.at[pl.ds(b * TQ, TQ), :], sem_in.at[b])

    def wcp(n):
        return pltpu.make_async_copy(wqkv_hbm.at[:, pl.ds(n * D, D)], wqkv_s.at[n], sem_in.at[NQ + n])

    late = [pltpu.make_async_copy(src, dst, sem_in.at[NQ + 3 + n])
            for n, (src, dst) in enumerate([(wo_hbm, wo_s), (wr_hbm, wr_s.at[pl.ds(0, D)]), (wg_hbm, wg_s),
                                            (wu_hbm, wu_s), (wd_hbm, wd_s)])]
    for cp in (xcp(0), wcp(1), xcp(1), wcp(0), wcp(2), xcp(2), xcp(3)):
        cp.start()

    def clear_drain():
        for k in range(NC - LAG, NC):
            c = PV_ORDER[k]
            p_s[(S + c * CK) // 2:(S + (c + 1) * CK) // 2, :] = jnp.zeros((CK // 2, TQ), u32)

    clear_drain()
    l_s[...] = jnp.ones((8, TQ), f32)
    acc_s[...] = jnp.ones((DH, TQ), f32)
    bad_s[...] = jnp.zeros((8, TQ), f32)
    w0_s[...] = jnp.zeros((64, TQ), u32)
    w1_s[...] = jnp.zeros((64, TQ), u32)
    ws = [w0_s, w1_s]

    def head_rows(h):
        return pl.ds(pl.multiple_of((h % 8) * 8, 8), 8)

    def prep_w(h, j, slot, h_old=None):
        qrows = qt_s[h // 8, j, head_rows(h), :]
        if h_old is not None:
            ws[slot][head_rows(h_old), :] = jnp.zeros((8, TQ), u32)
        ws[slot][head_rows(h), :] = qrows
        qf_s[slot] = _unpack(qrows).astype(f32)

    def gen_kb(h, kb, base, d, b, half):
        rowv = kt_s[h, d:d + 1, b * 128:(b + 1) * 128]
        if half:
            x = jnp.broadcast_to(rowv.astype(bf16), (128, 128)).T.astype(f32)
        else:
            x = jnp.broadcast_to(rowv, (128, 128)).T
        kb[base + d, b * 128:(b + 1) * 128, :] = x

    def ln1(b, dep=None):
        x = x_s[b * TQ:(b + 1) * TQ, :].astype(f32)
        if dep is not None:
            never = x_s[0:16, :].astype(f32)[0:8] > jnp.inf
            x = jnp.concatenate([jnp.where(never, dep[q:q + 8], x[q:q + 8]) for q in range(0, TQ, 8)], axis=0)
        return _ln(x).astype(bf16)

    def proj_k(b, xn):
        kf = jnp.dot(xn, wqkv_s[1], preferred_element_type=f32)
        k = kf.astype(bf16)
        for g in range(4):
            k_s.at[g][b * TQ // 2:(b + 1) * TQ // 2, :] = pltpu.bitcast(k[:, g * 128:(g + 1) * 128], u32)
        if b == 0:
            kt_s[...] = k[0:V].T.astype(f32).reshape(H, DH, V)
        return kf

    def proj_q(b, xn):
        qt = (jnp.dot(xn, wqkv_s[0], preferred_element_type=f32) * QSCALE).astype(bf16).T
        qt_s[:, b] = pltpu.bitcast(qt, u32).reshape(4, 64, TQ)

    def proj_v(b, xn):
        v = jnp.dot(xn, wqkv_s[2], preferred_element_type=f32)
        vmax = jnp.abs(v).reshape(TQ // 8, 8, D).max(axis=0)
        bad_s[...] = jnp.where(vmax <= V_HI, bad_s[...], 1.0)
        vt_s[:, :, b * TQ:(b + 1) * TQ] = pltpu.bitcast(v.astype(bf16).T, u32).reshape(H, 8, TQ)
        return v

    pre = [(n, d, b) for n in range(H // 2) for d, b in GENS]

    def pregen(n, total=9):
        for e, d, b in pre[(len(pre) * n) // total:(len(pre) * (n + 1)) // total]:
            gen_kb(2 * e, kbe_s, e * DH, d, b, True)

    xcp(0).wait()
    xn0 = ln1(0)
    wcp(1).wait()
    proj_k(0, xn0)
    xcp(1).wait()
    wcp(0).wait()
    proj_q(0, xn0)
    xn1 = ln1(1)
    proj_k(1, xn1)
    wcp(2).wait()
    xcp(2).wait()
    xcp(3).wait()
    for cp in late:
        cp.start()
    pregen(0)
    xn2 = ln1(2, proj_v(0, xn0))
    prep_w(0, 0, 0)
    pregen(1)
    proj_q(1, xn1)
    pregen(2)
    proj_v(1, xn1)
    pregen(3)
    xn3 = ln1(3, proj_k(2, xn2))
    pregen(4)
    proj_q(2, xn2)
    pregen(5)
    proj_v(2, xn2)
    pregen(6)
    proj_k(3, xn3)
    pregen(7)
    proj_q(3, xn3)
    pregen(8)
    proj_v(3, xn3)
    for cp in late:
        cp.wait()

    def finish_rows(slot, r0, s, l8):
        p = jnp.exp2(s)
        for r in range(0, s.shape[0], 16):
            t = p[r:r + 8] + p[r + 8:r + 16]
            l8 = t if l8 is None else l8 + t
        r0 = slot * S + r0
        p_s[r0 // 2:(r0 + s.shape[0]) // 2, :] = _pack(p)
        return l8

    def pv_chunk(h, slot, c, acc):
        r0 = slot * S + c * CK
        pv = jnp.dot(_unpack(vt_s[h, :, c * CK:(c + 1) * CK]), _unpack(p_s[r0 // 2:(r0 + CK) // 2, :]),
                     preferred_element_type=f32)
        return pv if acc is None else acc + pv

    def close_sum(l8):
        l = l8.sum(axis=0, keepdims=True)
        bad_s[...] = jnp.where((l >= L_LO) & (l <= L_HI), bad_s[...], 1.0)
        return l

    def fin(h, j, l8, acc):
        ot_s.at[j, h][...] = _pack(acc * (1.0 / close_sum(l8)))

    def body(i, carry):
        zero = jnp.minimum(i, 0)
        never = (lax.broadcasted_iota(jnp.int32, (16, 128), 0) + i) < 0
        lq = [l_s[...]]
        hist = []
        for hh in range(HPB):
            h = i * HPB + hh
            hprev = jnp.maximum(h - 1, 0) if hh == 0 else h - 1
            hnext = jnp.minimum(h + 1, H - 1) if hh == HPB - 1 else h + 1
            kbr, kbase = (kbe_s, (h // 2) * DH) if hh % 2 == 0 else (kbo_s, zero)
            for t in range(NQ):
                slot = t % 2
                l8 = None
                l8v = None
                vacc = None
                for c in range(NC):
                    r0, r1 = BOUNDS[c], BOUNDS[c + 1]
                    s = jnp.dot(_unpack(k_s[h // 8, r0 // 2:r1 // 2, :]), _unpack(ws[slot][...]),
                                preferred_element_type=f32)
                    base = len(hist)
                    hist.extend([s[r:r + 8, 0:128] for r in range(0, r1 - r0, 8)])
                    n_new = len(hist) - base
                    l8 = finish_rows(slot, r0, s, l8)
                    pcs = PIECES[(len(PIECES) * c) // NC:(len(PIECES) * (c + 1)) // NC]
                    for n, (vg, d) in enumerate(pcs):
                        kb = kbr[kbase + d, vg * 16:(vg + 1) * 16, :]
                        ii = base + (n * n_new) // len(pcs) - VOFF
                        if ii >= 0:
                            kb = jnp.where(never, jnp.concatenate([hist[ii]] * 2, axis=0), kb)
                        qb = jnp.concatenate(
                            [jnp.broadcast_to(qf_s.at[slot][d:d + 1, cc * 128:(cc + 1) * 128], (16, 128))
                             for cc in range(TQ // 128)], axis=1)
                        tt = jnp.concatenate([kb] * (TQ // 128), axis=1) * qb
                        vacc = tt if d == 0 else vacc + tt
                        if d == DH - 1:
                            l8v = finish_rows(slot, vg * 16, vacc, l8v)
                    rel, k = divmod(t * NC + c - LAG, NC)
                    hb = hprev if rel < 0 else h
                    acc = pv_chunk(hb, rel % 2, PV_ORDER[k], None if k == 0 else acc_s[...])
                    if k == NC - 1:
                        fin(hb, rel % NQ, lq.pop(0), acc)
                    else:
                        acc_s[...] = acc
                    if c == LAG:
                        if t + 1 < NQ:
                            prep_w(h, t + 1, 1 - slot, hprev if t == 0 else None)
                        else:
                            prep_w(hnext, 0, 1 - slot, h)
                    if hh % 2 == 0:
                        st = t * NC + c
                        for gi in range((len(GENS) * st) // (NQ * NC), (len(GENS) * (st + 1)) // (NQ * NC)):
                            gen_kb(hnext, kbo_s, 0, *GENS[gi], False)
                lq.append(l8 + l8v)
        l_s[...] = lq[0]
        return carry

    lax.fori_loop(0, H // HPB, body, 0)
    close_sum(l_s[...])

    @pl.when(jnp.max(bad_s[...]) > 0.0)
    def _():
        row = lax.broadcasted_iota(jnp.int32, (64, TQ), 0) // 8

        def unit(u, carry):
            h = u // NQ
            j = u % NQ
            w0_s[...] = jnp.where(row == (h % 8), qt_s[h // 8, j], jnp.uint32(0))

            def scores(c, m8):
                kc = _unpack(k_s[h // 8, pl.ds(pl.multiple_of(c * (CK // 2), CK // 2), CK // 2), :])
                s = jnp.dot(kc, _unpack(w0_s[...]), preferred_element_type=f32)
                s_s[pl.ds(pl.multiple_of(c * CK, CK), CK), :] = s
                return jnp.maximum(m8, s.reshape(CK // 8, 8, TQ).max(axis=0))

            m8 = lax.fori_loop(0, NC, scores, jnp.full((8, TQ), -jnp.inf, f32))
            m = m8.max(axis=0, keepdims=True)

            def probs(c, l8):
                p = jnp.exp2(s_s[pl.ds(pl.multiple_of(c * CK, CK), CK), :] - m)
                p_s[pl.ds(pl.multiple_of(c * (CK // 2), CK // 2), CK // 2), :] = _pack(p)
                return l8 + p.reshape(CK // 8, 8, TQ).sum(axis=0)

            l8 = lax.fori_loop(0, NC, probs, jnp.zeros((8, TQ), f32))
            o = jnp.dot(_unpack(vt_s[h]), _unpack(p_s[0:S // 2, :]), preferred_element_type=f32)
            o = o * (1.0 / l8.sum(axis=0, keepdims=True))
            ot_s[j, h] = _pack(o)
            acc_s[...] = o
            return carry

        lax.fori_loop(0, H * NQ, unit, 0)
        clear_drain()
        l_s[...] = jnp.full((8, TQ), 0.125, f32)

    acc = acc_s[...]
    for k in range(NC - LAG, NC):
        acc = pv_chunk(H - 1, 1, PV_ORDER[k], acc)
    fin(H - 1, NQ - 1, l_s[...], acc)

    w4 = wr_s[0:D].reshape(4, 128).astype(f32)
    wr16 = jnp.concatenate([jnp.broadcast_to(w4[j:j + 1], (16, 128)) for j in range(4)], axis=1).astype(bf16)

    def oproj(n):
        b, lo = divmod(n * EB, TQ)
        o = _unpack(ot_s[b, :, :, lo:lo + EB].reshape(H * 8, EB)).T
        return jnp.dot(o, wo_s[...], preferred_element_type=f32)

    def post(n, a):
        r0 = n * EB
        h = x_s[r0:r0 + EB, :].astype(f32) + a
        hn = _ln(h)
        out_s[r0:r0 + EB, :] = (h + hn).astype(bf16)
        hn_s[r0 // 2:(r0 + EB) // 2, :] = _pack(hn)

    def router(n):
        r0 = n * EB
        r = lax.dot_general(wr16, _unpack(hn_s[r0 // 2:(r0 + EB) // 2, :]), (((1,), (1,)), ((), ())),
                            preferred_element_type=f32)
        r_s[:, r0:r0 + EB] = r[0:8]

    ocps = []

    def send(r0, r1):
        cp = pltpu.make_async_copy(out_s.at[pl.ds(r0, r1 - r0), :], out_hbm.at[pl.ds(r0, r1 - r0), :],
                                   sem_out.at[len(ocps)])
        cp.start()
        ocps.append(cp)
        return r1

    nsub = S // EB
    sent = 0
    a_next = oproj(0)
    for n in range(nsub):
        a_cur = a_next
        if n + 1 < nsub:
            a_next = oproj(n + 1)
        if n in OUT_STARTS:
            sent = send(sent, n * EB)
        if n > 0:
            router(n - 1)
        post(n, a_cur)
    send(sent, S)
    router(nsub - 1)

    bits = pltpu.bitcast(r_s[...].astype(bf16).astype(f32), jnp.int32)
    idx = lax.broadcasted_iota(jnp.int32, (8, S), 1)
    key = ((bits ^ ((bits >> 31) & 0x7FFFFFFF)) & -65536) | (S - 1 - idx)
    k1 = jnp.max(key, axis=1, keepdims=True)
    k2 = jnp.max(jnp.where(key == k1, jnp.iinfo(jnp.int32).min, key), axis=1, keepdims=True)
    i1 = S - 1 - (k1[0, 0] & (S - 1))
    i2 = S - 1 - (k2[0, 0] & (S - 1))

    def gate(k):
        hi = k & -65536
        r = pltpu.bitcast(jnp.broadcast_to((hi ^ ((hi >> 31) & 0x7FFFFFFF)) & -65536, (8, 128)), f32)[0:1, 0:1]
        return jax.nn.sigmoid(r)

    t1 = pl.multiple_of((i1 // 16) * 16, 16)
    t2 = pl.multiple_of((i2 // 16) * 16, 16)
    xs = _unpack(jnp.concatenate([hn_s[pl.ds(pl.multiple_of(t // 2, 8), 8), :] for t in (t1, t2)], axis=0))
    g = jnp.dot(xs, wg_s[...], preferred_element_type=f32)
    u = jnp.dot(xs, wu_s[...], preferred_element_type=f32)
    y = jnp.dot((g * jax.nn.sigmoid(g) * u).astype(bf16), wd_s[...], preferred_element_type=f32)
    s1 = gate(k1)
    s2 = gate(k2)
    rows16 = lax.broadcasted_iota(jnp.int32, (16, D), 0)
    for n, t in enumerate((t1, t2)):
        rid = rows16 + t
        yt = y[n * 16:(n + 1) * 16]
        upd = jnp.where(rid == i1, yt * s1, jnp.where(rid == i2, yt * s2, 0.0))
        patch_s[n] = (out_s[pl.ds(t, 16), :].astype(f32) + upd).astype(bf16)
    for cp in ocps:
        cp.wait()
    p1 = pltpu.make_async_copy(patch_s.at[0], out_hbm.at[pl.ds(t1, 16), :], sem_out.at[len(ocps)])
    p2 = pltpu.make_async_copy(patch_s.at[1], out_hbm.at[pl.ds(t2, 16), :], sem_out.at[len(ocps) + 1])
    p1.start()

    @pl.when(t1 != t2)
    def _():
        p2.start()
        p2.wait()

    p1.wait()


@jax.jit
def pallas_sequential_preLN__mha_block__moe_arch_mod__prompt_kernel(
    A_x: jax.Array,
    A_wqkv: jax.Array,
    A_wo: jax.Array,
    B_x: jax.Array,
    B_w_r: jax.Array,
    B_w_gate: jax.Array,
    B_w_up: jax.Array,
    B_w_down: jax.Array,
):
    del B_x
    any_spec = pl.BlockSpec(memory_space=pl.ANY)
    out = pl.pallas_call(
        _kernel,
        out_shape=jax.ShapeDtypeStruct((S, D), bf16),
        in_specs=[any_spec] * 7,
        out_specs=any_spec,
        scratch_shapes=[
            pltpu.VMEM((S, D), bf16),
            pltpu.VMEM((3, D, D), bf16),
            pltpu.VMEM((D, D), bf16),
            pltpu.VMEM((D, F), bf16),
            pltpu.VMEM((D, F), bf16),
            pltpu.VMEM((F, D), bf16),
            pltpu.VMEM((4, S // 2, 128), u32),
            pltpu.VMEM((4, NQ, 64, TQ), u32),
            pltpu.VMEM((H, 8, S), u32),
            pltpu.VMEM((NQ, H, 8, TQ), u32),
            pltpu.VMEM((H, DH, V), f32),
            pltpu.VMEM((H // 2 * DH, V, 128), f32),
            pltpu.VMEM((DH, V, 128), f32),
            pltpu.VMEM((2, DH, TQ), f32),
            pltpu.VMEM((S, TQ), u32),
            pltpu.VMEM((64, TQ), u32),
            pltpu.VMEM((64, TQ), u32),
            pltpu.VMEM((8, TQ), f32),
            pltpu.VMEM((DH, TQ), f32),
            pltpu.VMEM((8, TQ), f32),
            pltpu.VMEM((S // 2, D), u32),
            pltpu.VMEM((S, TQ), f32),
            pltpu.VMEM((S, D), bf16),
            pltpu.VMEM((8, S), f32),
            pltpu.VMEM((2, 16, D), bf16),
            pltpu.VMEM((4 * D,), bf16),
            pltpu.SemaphoreType.DMA((NQ + 8,)),
            pltpu.SemaphoreType.DMA((len(OUT_STARTS) + 3,)),
        ],
        compiler_params=pltpu.CompilerParams(vmem_limit_bytes=100 * 1024 * 1024),
    )(A_x.reshape(S, D), A_wqkv, A_wo, B_w_r, B_w_gate, B_w_up, B_w_down)
    return out.reshape(1, S, D)
```

```python
import math

import jax
import jax.numpy as jnp
from jax import lax
import jax.experimental.pallas as pl
import jax.experimental.pallas.tpu as pltpu

f32 = jnp.float32
bf16 = jnp.bfloat16
u32 = jnp.uint32

S = 2048
D = 512
H = 32
DH = 16
F = 1792
TQ = 512
NQ = S // TQ
CK = 128
NC = S // CK
NV = 16
V = NV * 16
VB = V // 128
LAG = 4
VOFF = 4
HPB = 2
EB = 256
OUT_STARTS = (4, 7)
EPS = 1e-5
QSCALE = (DH ** -0.5) * math.log2(math.e)
L_LO = 2.0 ** -40
L_HI = 2.0 ** 64
KEY0 = 0x20000000
V_HI = 2.0 ** 60

PV_ORDER = list(range(VB, NC)) + list(range(VB))
BOUNDS = [V + 16 * ((((S - V) // 16) * c) // NC) for c in range(NC + 1)]
PIECES = [(vg, d) for vg in range(NV) for d in range(DH)]
GENS = [(d, b) for b in range(VB) for d in range(DH)]


def _ln(x):
    mu = jnp.mean(x, axis=-1, keepdims=True)
    xc = x - mu
    var = jnp.mean(xc * xc, axis=-1, keepdims=True)
    return xc * lax.rsqrt(var + EPS)


def _pack(x):
    return pltpu.bitcast(x.astype(bf16), u32)


def _mm(x, w_ref):
    a = None
    for c in range(0, x.shape[1], 128):
        t = jnp.dot(x[:, c:c + 128], w_ref[c:c + 128, :], preferred_element_type=f32)
        a = t if a is None else a + t
    return a


def _unpack(x):
    return pltpu.bitcast(x, bf16)


def _kernel(x_hbm, wqkv_hbm, wo_hbm, wr_hbm, wg_hbm, wu_hbm, wd_hbm, out_hbm,
            x_s, wqkv_s, wo_s, wg_s, wu_s, wd_s,
            k_s, qt_s, vt_s, ot_s, kt_s, kbe_s, kbo_s, qf_s, p_s, w0_s, w1_s, l_s, acc_s, bad_s,
            hn_s, s_s, out_s, patch_s, wr_s, sem_in, sem_out):
    def xcp(b):
        return pltpu.make_async_copy(x_hbm.at[pl.ds(b * TQ, TQ), :], x_s.at[pl.ds(b * TQ, TQ), :], sem_in.at[b])

    def wcp(n):
        return pltpu.make_async_copy(wqkv_hbm.at[:, pl.ds(n * D, D)], wqkv_s.at[n], sem_in.at[NQ + n])

    late = [pltpu.make_async_copy(src, dst, sem_in.at[NQ + 3 + n])
            for n, (src, dst) in enumerate([(wo_hbm, wo_s), (wr_hbm, wr_s.at[pl.ds(0, D)]), (wg_hbm, wg_s),
                                            (wu_hbm, wu_s), (wd_hbm, wd_s)])]
    for cp in (xcp(0), wcp(1), xcp(1), wcp(0), wcp(2), xcp(2), xcp(3)):
        cp.start()

    def clear_drain():
        for k in range(NC - LAG, NC):
            c = PV_ORDER[k]
            p_s[(S + c * CK) // 2:(S + (c + 1) * CK) // 2, :] = jnp.zeros((CK // 2, TQ), u32)

    clear_drain()
    l_s[...] = jnp.ones((8, TQ), f32)
    acc_s[...] = jnp.ones((DH, TQ), f32)
    bad_s[...] = jnp.zeros((8, TQ), f32)
    w0_s[...] = jnp.zeros((64, TQ), u32)
    w1_s[...] = jnp.zeros((64, TQ), u32)
    ws = [w0_s, w1_s]

    def head_rows(h):
        return pl.ds(pl.multiple_of((h % 8) * 8, 8), 8)

    def prep_w(h, j, slot, h_old=None):
        qrows = qt_s[h // 8, j, head_rows(h), :]
        if h_old is not None:
            ws[slot][head_rows(h_old), :] = jnp.zeros((8, TQ), u32)
        ws[slot][head_rows(h), :] = qrows
        qf_s[slot] = _unpack(qrows).astype(f32)

    def gen_kb(h, kb, base, d, b, half):
        rowv = kt_s[h, d:d + 1, b * 128:(b + 1) * 128]
        if half:
            x = jnp.broadcast_to(rowv.astype(bf16), (128, 128)).T.astype(f32)
        else:
            x = jnp.broadcast_to(rowv, (128, 128)).T
        kb[base + d, b * 128:(b + 1) * 128, :] = x

    def ln1(b, dep=None):
        x = x_s[b * TQ:(b + 1) * TQ, :].astype(f32)
        if dep is not None:
            never = x_s[0:16, :].astype(f32)[0:8] > jnp.inf
            x = jnp.concatenate([jnp.where(never, dep[q:q + 8], x[q:q + 8]) for q in range(0, TQ, 8)], axis=0)
        return _ln(x).astype(bf16)

    def proj_k(b, xn):
        kf = jnp.dot(xn, wqkv_s[1], preferred_element_type=f32)
        k = kf.astype(bf16)
        for g in range(4):
            k_s.at[g][b * TQ // 2:(b + 1) * TQ // 2, :] = pltpu.bitcast(k[:, g * 128:(g + 1) * 128], u32)
        if b == 0:
            kt_s[...] = k[0:V].T.astype(f32).reshape(H, DH, V)
        return kf

    def proj_q(b, xn):
        qt = (jnp.dot(xn, wqkv_s[0], preferred_element_type=f32) * QSCALE).astype(bf16).T
        qt_s[:, b] = pltpu.bitcast(qt, u32).reshape(4, 64, TQ)

    def proj_v(b, xn):
        v = jnp.dot(xn, wqkv_s[2], preferred_element_type=f32)
        vmax = jnp.abs(v).reshape(TQ // 8, 8, D).max(axis=0)
        bad_s[...] = jnp.where(vmax <= V_HI, bad_s[...], 1.0)
        vt_s[:, :, b * TQ:(b + 1) * TQ] = pltpu.bitcast(v.astype(bf16).T, u32).reshape(H, 8, TQ)
        return v

    pre = [(n, d, b) for n in range(H // 2) for d, b in GENS]

    def pregen(n, total=9):
        for e, d, b in pre[(len(pre) * n) // total:(len(pre) * (n + 1)) // total]:
            gen_kb(2 * e, kbe_s, e * DH, d, b, True)

    xcp(0).wait()
    xn0 = ln1(0)
    wcp(1).wait()
    proj_k(0, xn0)
    xcp(1).wait()
    wcp(0).wait()
    proj_q(0, xn0)
    xn1 = ln1(1)
    proj_k(1, xn1)
    wcp(2).wait()
    xcp(2).wait()
    xcp(3).wait()
    for cp in late:
        cp.start()
    pregen(0)
    xn2 = ln1(2, proj_v(0, xn0))
    prep_w(0, 0, 0)
    pregen(1)
    proj_q(1, xn1)
    pregen(2)
    proj_v(1, xn1)
    pregen(3)
    xn3 = ln1(3, proj_k(2, xn2))
    pregen(4)
    proj_q(2, xn2)
    pregen(5)
    proj_v(2, xn2)
    pregen(6)
    proj_v(3, xn3)
    pregen(7)
    proj_q(3, xn3)
    pregen(8)
    proj_k(3, xn3)
    for cp in late:
        cp.wait()

    def finish_rows(slot, r0, s, l8):
        p = jnp.exp2(s)
        for r in range(0, s.shape[0], 16):
            t = p[r:r + 8] + p[r + 8:r + 16]
            l8 = t if l8 is None else l8 + t
        r0 = slot * S + r0
        p_s[r0 // 2:(r0 + s.shape[0]) // 2, :] = _pack(p)
        return l8

    def pv_chunk(h, slot, c, acc):
        r0 = slot * S + c * CK
        pv = jnp.dot(_unpack(vt_s[h, :, c * CK:(c + 1) * CK]), _unpack(p_s[r0 // 2:(r0 + CK) // 2, :]),
                     preferred_element_type=f32)
        return pv if acc is None else acc + pv

    def close_sum(l8):
        l = l8.sum(axis=0, keepdims=True)
        bad_s[...] = jnp.where((l >= L_LO) & (l <= L_HI), bad_s[...], 1.0)
        return l

    def fin(h, j, l8, acc):
        ot_s.at[j, h][...] = _pack(acc * (1.0 / close_sum(l8)))

    def body(i, carry):
        zero = jnp.minimum(i, 0)
        never = (lax.broadcasted_iota(jnp.int32, (16, 128), 0) + i) < 0
        lq = [l_s[...]]
        hist = []
        for hh in range(HPB):
            h = i * HPB + hh
            hprev = jnp.maximum(h - 1, 0) if hh == 0 else h - 1
            hnext = jnp.minimum(h + 1, H - 1) if hh == HPB - 1 else h + 1
            kbr, kbase = (kbe_s, (h // 2) * DH) if hh % 2 == 0 else (kbo_s, zero)
            for t in range(NQ):
                slot = t % 2
                l8 = None
                l8v = None
                vacc = None
                for c in range(NC):
                    r0, r1 = BOUNDS[c], BOUNDS[c + 1]
                    s = jnp.dot(_unpack(k_s[h // 8, r0 // 2:r1 // 2, :]), _unpack(ws[slot][...]),
                                preferred_element_type=f32)
                    base = len(hist)
                    hist.extend([s[r:r + 8, 0:128] for r in range(0, r1 - r0, 8)])
                    n_new = len(hist) - base
                    l8 = finish_rows(slot, r0, s, l8)
                    pcs = PIECES[(len(PIECES) * c) // NC:(len(PIECES) * (c + 1)) // NC]
                    for n, (vg, d) in enumerate(pcs):
                        kb = kbr[kbase + d, vg * 16:(vg + 1) * 16, :]
                        ii = base + (n * n_new) // len(pcs) - VOFF
                        if ii >= 0:
                            kb = jnp.where(never, jnp.concatenate([hist[ii]] * 2, axis=0), kb)
                        qb = jnp.concatenate(
                            [jnp.broadcast_to(qf_s.at[slot][d:d + 1, cc * 128:(cc + 1) * 128], (16, 128))
                             for cc in range(TQ // 128)], axis=1)
                        tt = jnp.concatenate([kb] * (TQ // 128), axis=1) * qb
                        vacc = tt if d == 0 else vacc + tt
                        if d == DH - 1:
                            l8v = finish_rows(slot, vg * 16, vacc, l8v)
                    rel, k = divmod(t * NC + c - LAG, NC)
                    hb = hprev if rel < 0 else h
                    acc = pv_chunk(hb, rel % 2, PV_ORDER[k], None if k == 0 else acc_s[...])
                    if k == NC - 1:
                        fin(hb, rel % NQ, lq.pop(0), acc)
                    else:
                        acc_s[...] = acc
                    if c == LAG:
                        if t + 1 < NQ:
                            prep_w(h, t + 1, 1 - slot, hprev if t == 0 else None)
                        else:
                            prep_w(hnext, 0, 1 - slot, h)
                    if hh % 2 == 0:
                        st = t * NC + c
                        for gi in range((len(GENS) * st) // (NQ * NC), (len(GENS) * (st + 1)) // (NQ * NC)):
                            gen_kb(hnext, kbo_s, 0, *GENS[gi], False)
                lq.append(l8 + l8v)
        l_s[...] = lq[0]
        return carry

    lax.fori_loop(0, H // HPB, body, 0)
    close_sum(l_s[...])

    @pl.when(jnp.max(bad_s[...]) > 0.0)
    def _():
        row = lax.broadcasted_iota(jnp.int32, (64, TQ), 0) // 8

        def unit(u, carry):
            h = u // NQ
            j = u % NQ
            w0_s[...] = jnp.where(row == (h % 8), qt_s[h // 8, j], jnp.uint32(0))

            def scores(c, m8):
                kc = _unpack(k_s[h // 8, pl.ds(pl.multiple_of(c * (CK // 2), CK // 2), CK // 2), :])
                s = jnp.dot(kc, _unpack(w0_s[...]), preferred_element_type=f32)
                s_s[pl.ds(pl.multiple_of(c * CK, CK), CK), :] = s
                return jnp.maximum(m8, s.reshape(CK // 8, 8, TQ).max(axis=0))

            m8 = lax.fori_loop(0, NC, scores, jnp.full((8, TQ), -jnp.inf, f32))
            m = m8.max(axis=0, keepdims=True)

            def probs(c, l8):
                p = jnp.exp2(s_s[pl.ds(pl.multiple_of(c * CK, CK), CK), :] - m)
                p_s[pl.ds(pl.multiple_of(c * (CK // 2), CK // 2), CK // 2), :] = _pack(p)
                return l8 + p.reshape(CK // 8, 8, TQ).sum(axis=0)

            l8 = lax.fori_loop(0, NC, probs, jnp.zeros((8, TQ), f32))
            o = jnp.dot(_unpack(vt_s[h]), _unpack(p_s[0:S // 2, :]), preferred_element_type=f32)
            o = o * (1.0 / l8.sum(axis=0, keepdims=True))
            ot_s[j, h] = _pack(o)
            acc_s[...] = o
            return carry

        lax.fori_loop(0, H * NQ, unit, 0)
        clear_drain()
        l_s[...] = jnp.full((8, TQ), 0.125, f32)

    acc = acc_s[...]
    for k in range(NC - LAG, NC):
        acc = pv_chunk(H - 1, 1, PV_ORDER[k], acc)
    fin(H - 1, NQ - 1, l_s[...], acc)

    w4 = wr_s[0:D].reshape(4, 128).astype(f32)
    wrow = jnp.concatenate([w4[j:j + 1] for j in range(4)], axis=1)
    wr16 = jnp.broadcast_to(wrow, (16, D)).astype(bf16)
    top = []
    topl = []
    nsub = S // EB

    def oproj(n):
        b, lo = divmod(n * EB, TQ)
        o = _unpack(ot_s[b, :, :, lo:lo + EB].reshape(H * 8, EB)).T
        return _mm(o, wo_s)

    def merge(a, b):
        return jnp.maximum(a[0], b[0]), jnp.maximum(jnp.minimum(a[0], b[0]), jnp.maximum(a[1], b[1]))

    def route_key(r, tok):
        bits = pltpu.bitcast(r.astype(bf16).astype(f32), jnp.int32)
        code = ((bits ^ ((bits >> 31) & 0x7FFFFFFF)) >> 16) + 32768
        return pltpu.bitcast(KEY0 + code * S + (S - 1 - tok), f32)

    def push(acc, a, b):
        pair = jnp.maximum(a, b), jnp.minimum(a, b)
        acc[:] = [merge(acc[0], pair)] if acc else [pair]

    def post(n, a):
        r0 = n * EB
        h = x_s[r0:r0 + EB, :].astype(f32) + a
        hn = _ln(h)
        out_s[r0:r0 + EB, :] = (h + hn).astype(bf16)
        hn_s[r0 // 2:(r0 + EB) // 2, :] = _pack(hn)
        if n == nsub - 1:
            r = jnp.sum(hn.astype(bf16).astype(f32) * wrow, axis=1, keepdims=True)
            key = route_key(jnp.broadcast_to(r, (EB, 128)), r0 + lax.broadcasted_iota(jnp.int32, (EB, 128), 0))
            for q in range(0, EB, 16):
                push(top, key[q:q + 8], key[q + 8:q + 16])

    def router(n):
        r0 = n * EB
        r = lax.dot_general(wr16, _unpack(hn_s[r0 // 2:(r0 + EB) // 2, :]), (((1,), (1,)), ((), ())),
                            preferred_element_type=f32)[0:8]
        key = route_key(r, r0 + lax.broadcasted_iota(jnp.int32, (8, EB), 1))
        for q in range(0, EB, 256):
            push(topl, key[:, q:q + 128], key[:, q + 128:q + 256])

    ocps = []

    def send(r0, r1):
        cp = pltpu.make_async_copy(out_s.at[pl.ds(r0, r1 - r0), :], out_hbm.at[pl.ds(r0, r1 - r0), :],
                                   sem_out.at[len(ocps)])
        cp.start()
        ocps.append(cp)
        return r1

    sent = 0
    a_next = oproj(0)
    for n in range(nsub):
        a_cur = a_next
        if n + 1 < nsub:
            a_next = oproj(n + 1)
        if n in OUT_STARTS:
            sent = send(sent, n * EB)
        if n > 0:
            router(n - 1)
        post(n, a_cur)
    send(sent, S)

    best = top[0]
    for sh in (4, 2, 1):
        best = merge(best, (pltpu.roll(best[0], sh, 0), pltpu.roll(best[1], sh, 0)))
    l1 = jnp.max(topl[0][0], axis=1, keepdims=True)
    l2 = jnp.max(jnp.where(topl[0][0] == l1, topl[0][1], topl[0][0]), axis=1, keepdims=True)
    best = merge(best, (jnp.broadcast_to(l1, (8, 128)), jnp.broadcast_to(l2, (8, 128))))
    k1 = pltpu.bitcast(best[0], jnp.int32) - KEY0
    k2 = pltpu.bitcast(best[1], jnp.int32) - KEY0
    i1 = S - 1 - (k1[0, 0] & (S - 1))
    i2 = S - 1 - (k2[0, 0] & (S - 1))

    def gate(k):
        hi = ((k >> 11) - 32768) << 16
        r = pltpu.bitcast((hi ^ ((hi >> 31) & 0x7FFFFFFF)) & -65536, f32)[0:1, 0:1]
        return jax.nn.sigmoid(r)

    t1 = pl.multiple_of((i1 // 16) * 16, 16)
    t2 = pl.multiple_of((i2 // 16) * 16, 16)
    xs = _unpack(jnp.concatenate([hn_s[pl.ds(pl.multiple_of(t // 2, 8), 8), :] for t in (t1, t2)], axis=0))
    g = jnp.dot(xs, wg_s[...], preferred_element_type=f32)
    u = jnp.dot(xs, wu_s[...], preferred_element_type=f32)
    y = jnp.dot((g * jax.nn.sigmoid(g) * u).astype(bf16), wd_s[...], preferred_element_type=f32)
    s1 = gate(k1)
    s2 = gate(k2)
    rows16 = lax.broadcasted_iota(jnp.int32, (16, D), 0)
    for n, t in enumerate((t1, t2)):
        rid = rows16 + t
        yt = y[n * 16:(n + 1) * 16]
        upd = jnp.where(rid == i1, yt * s1, jnp.where(rid == i2, yt * s2, 0.0))
        patch_s[n] = (out_s[pl.ds(t, 16), :].astype(f32) + upd).astype(bf16)
    for cp in ocps:
        cp.wait()
    p1 = pltpu.make_async_copy(patch_s.at[0], out_hbm.at[pl.ds(t1, 16), :], sem_out.at[len(ocps)])
    p2 = pltpu.make_async_copy(patch_s.at[1], out_hbm.at[pl.ds(t2, 16), :], sem_out.at[len(ocps) + 1])
    p1.start()

    @pl.when(t1 != t2)
    def _():
        p2.start()
        p2.wait()

    p1.wait()


@jax.jit
def pallas_sequential_preLN__mha_block__moe_arch_mod__prompt_kernel(
    A_x: jax.Array,
    A_wqkv: jax.Array,
    A_wo: jax.Array,
    B_x: jax.Array,
    B_w_r: jax.Array,
    B_w_gate: jax.Array,
    B_w_up: jax.Array,
    B_w_down: jax.Array,
):
    del B_x
    any_spec = pl.BlockSpec(memory_space=pl.ANY)
    out = pl.pallas_call(
        _kernel,
        out_shape=jax.ShapeDtypeStruct((S, D), bf16),
        in_specs=[any_spec] * 7,
        out_specs=any_spec,
        scratch_shapes=[
            pltpu.VMEM((S, D), bf16),
            pltpu.VMEM((3, D, D), bf16),
            pltpu.VMEM((D, D), bf16),
            pltpu.VMEM((D, F), bf16),
            pltpu.VMEM((D, F), bf16),
            pltpu.VMEM((F, D), bf16),
            pltpu.VMEM((4, S // 2, 128), u32),
            pltpu.VMEM((4, NQ, 64, TQ), u32),
            pltpu.VMEM((H, 8, S), u32),
            pltpu.VMEM((NQ, H, 8, TQ), u32),
            pltpu.VMEM((H, DH, V), f32),
            pltpu.VMEM((H // 2 * DH, V, 128), f32),
            pltpu.VMEM((DH, V, 128), f32),
            pltpu.VMEM((2, DH, TQ), f32),
            pltpu.VMEM((S, TQ), u32),
            pltpu.VMEM((64, TQ), u32),
            pltpu.VMEM((64, TQ), u32),
            pltpu.VMEM((8, TQ), f32),
            pltpu.VMEM((DH, TQ), f32),
            pltpu.VMEM((8, TQ), f32),
            pltpu.VMEM((S // 2, D), u32),
            pltpu.VMEM((S, TQ), f32),
            pltpu.VMEM((S, D), bf16),
            pltpu.VMEM((2, 16, D), bf16),
            pltpu.VMEM((4 * D,), bf16),
            pltpu.SemaphoreType.DMA((NQ + 8,)),
            pltpu.SemaphoreType.DMA((len(OUT_STARTS) + 3,)),
        ],
        compiler_params=pltpu.CompilerParams(vmem_limit_bytes=100 * 1024 * 1024),
    )(A_x.reshape(S, D), A_wqkv, A_wo, B_w_r, B_w_gate, B_w_up, B_w_down)
    return out.reshape(1, S, D)
```

```python
import math

import jax
import jax.numpy as jnp
from jax import lax
import jax.experimental.pallas as pl
import jax.experimental.pallas.tpu as pltpu

f32 = jnp.float32
bf16 = jnp.bfloat16
u32 = jnp.uint32

S = 2048
D = 512
H = 32
DH = 16
F = 1792
TQ = 512
NQ = S // TQ
CK = 128
NC = S // CK
NV = 16
V = NV * 16
VB = V // 128
LAG = 4
VOFF = 4
HPB = 2
EB = 256
OUT_STARTS = (4, 7)
EPS = 1e-5
QSCALE = (DH ** -0.5) * math.log2(math.e)
L_LO = 2.0 ** -40
L_HI = 2.0 ** 30
KEY0 = 0x20000000
V_HI = 2.0 ** 60

PV_ORDER = list(range(VB, NC)) + list(range(VB))
BOUNDS = [V + 16 * ((((S - V) // 16) * c) // NC) for c in range(NC + 1)]
PIECES = [(vg, d) for vg in range(NV) for d in range(DH)]
GENS = [(d, b) for b in range(VB) for d in range(DH)]


def _ln(x):
    mu = jnp.mean(x, axis=-1, keepdims=True)
    xc = x - mu
    var = jnp.mean(xc * xc, axis=-1, keepdims=True)
    return xc * lax.rsqrt(var + EPS)


def _pack(x):
    return pltpu.bitcast(x.astype(bf16), u32)


def _mm(x, w_ref):
    a = None
    for c in range(0, x.shape[1], 128):
        t = jnp.dot(x[:, c:c + 128], w_ref[c:c + 128, :], preferred_element_type=f32)
        a = t if a is None else a + t
    return a


def _unpack(x):
    return pltpu.bitcast(x, bf16)


def _kernel(x_hbm, wqkv_hbm, wo_hbm, wr_hbm, wg_hbm, wu_hbm, wd_hbm, out_hbm,
            x_s, wqkv_s, wo_s, wg_s, wu_s, wd_s,
            k_s, qt_s, vt_s, ot_s, kt_s, kbe_s, kbo_s, qf_s, p_s, w0_s, w1_s, l_s, acc_s, bad_s,
            hn_s, s_s, klo_s, qlo_s, out_s, patch_s, wr_s, sem_in, sem_out):
    def xcp(b):
        return pltpu.make_async_copy(x_hbm.at[pl.ds(b * TQ, TQ), :], x_s.at[pl.ds(b * TQ, TQ), :], sem_in.at[b])

    def wcp(n):
        return pltpu.make_async_copy(wqkv_hbm.at[:, pl.ds(n * D, D)], wqkv_s.at[n], sem_in.at[NQ + n])

    late = [pltpu.make_async_copy(src, dst, sem_in.at[NQ + 3 + n])
            for n, (src, dst) in enumerate([(wo_hbm, wo_s), (wr_hbm, wr_s.at[pl.ds(0, D)]), (wg_hbm, wg_s),
                                            (wu_hbm, wu_s), (wd_hbm, wd_s)])]
    for cp in (xcp(0), wcp(1), xcp(1), wcp(0), wcp(2), xcp(2), xcp(3)):
        cp.start()

    def clear_drain():
        for k in range(NC - LAG, NC):
            c = PV_ORDER[k]
            p_s[(S + c * CK) // 2:(S + (c + 1) * CK) // 2, :] = jnp.zeros((CK // 2, TQ), u32)

    clear_drain()
    l_s[...] = jnp.ones((8, TQ), f32)
    acc_s[...] = jnp.ones((DH, TQ), f32)
    bad_s[...] = jnp.zeros((8, TQ), f32)
    w0_s[...] = jnp.zeros((64, TQ), u32)
    w1_s[...] = jnp.zeros((64, TQ), u32)
    ws = [w0_s, w1_s]

    def head_rows(h):
        return pl.ds(pl.multiple_of((h % 8) * 8, 8), 8)

    def prep_w(h, j, slot, h_old=None):
        qrows = qt_s[h // 8, j, head_rows(h), :]
        if h_old is not None:
            ws[slot][head_rows(h_old), :] = jnp.zeros((8, TQ), u32)
        ws[slot][head_rows(h), :] = qrows
        qf_s[slot] = _unpack(qrows).astype(f32)

    def gen_kb(h, kb, base, d, b, half):
        rowv = kt_s[h, d:d + 1, b * 128:(b + 1) * 128]
        if half:
            x = jnp.broadcast_to(rowv.astype(bf16), (128, 128)).T.astype(f32)
        else:
            x = jnp.broadcast_to(rowv, (128, 128)).T
        kb[base + d, b * 128:(b + 1) * 128, :] = x

    def ln1(b, dep=None):
        x = x_s[b * TQ:(b + 1) * TQ, :].astype(f32)
        if dep is not None:
            never = x_s[0:16, :].astype(f32)[0:8] > jnp.inf
            x = jnp.concatenate([jnp.where(never, dep[q:q + 8], x[q:q + 8]) for q in range(0, TQ, 8)], axis=0)
        return _ln(x).astype(bf16)

    def proj_k(b, xn):
        kf = jnp.dot(xn, wqkv_s[1], preferred_element_type=f32)
        k = kf.astype(bf16)
        for g in range(4):
            k_s.at[g][b * TQ // 2:(b + 1) * TQ // 2, :] = pltpu.bitcast(k[:, g * 128:(g + 1) * 128], u32)
        if b == 0:
            kt_s[...] = k[0:V].T.astype(f32).reshape(H, DH, V)
        return kf

    def proj_q(b, xn):
        qt = (jnp.dot(xn, wqkv_s[0], preferred_element_type=f32) * QSCALE).astype(bf16).T
        qt_s[:, b] = pltpu.bitcast(qt, u32).reshape(4, 64, TQ)

    def proj_v(b, xn):
        v = jnp.dot(xn, wqkv_s[2], preferred_element_type=f32)
        vmax = jnp.abs(v).reshape(TQ // 8, 8, D).max(axis=0)
        bad_s[...] = jnp.where(vmax <= V_HI, bad_s[...], 1.0)
        vt_s[:, :, b * TQ:(b + 1) * TQ] = pltpu.bitcast(v.astype(bf16).T, u32).reshape(H, 8, TQ)
        return v

    pre = [(n, d, b) for n in range(H // 2) for d, b in GENS]

    def pregen(n, total=9):
        for e, d, b in pre[(len(pre) * n) // total:(len(pre) * (n + 1)) // total]:
            gen_kb(2 * e, kbe_s, e * DH, d, b, True)

    xcp(0).wait()
    xn0 = ln1(0)
    wcp(1).wait()
    proj_k(0, xn0)
    xcp(1).wait()
    wcp(0).wait()
    proj_q(0, xn0)
    xn1 = ln1(1)
    proj_k(1, xn1)
    wcp(2).wait()
    xcp(2).wait()
    xcp(3).wait()
    for cp in late:
        cp.start()
    pregen(0)
    xn2 = ln1(2, proj_v(0, xn0))
    prep_w(0, 0, 0)
    pregen(1)
    proj_q(1, xn1)
    pregen(2)
    proj_v(1, xn1)
    pregen(3)
    xn3 = ln1(3, proj_k(2, xn2))
    pregen(4)
    proj_q(2, xn2)
    pregen(5)
    proj_v(2, xn2)
    pregen(6)
    proj_v(3, xn3)
    pregen(7)
    proj_q(3, xn3)
    pregen(8)
    proj_k(3, xn3)
    for cp in late:
        cp.wait()

    def finish_rows(slot, r0, s, l8):
        p = jnp.exp2(s)
        for r in range(0, s.shape[0], 16):
            t = p[r:r + 8] + p[r + 8:r + 16]
            l8 = t if l8 is None else l8 + t
        r0 = slot * S + r0
        p_s[r0 // 2:(r0 + s.shape[0]) // 2, :] = _pack(p)
        return l8

    def pv_chunk(h, slot, c, acc):
        r0 = slot * S + c * CK
        pv = jnp.dot(_unpack(vt_s[h, :, c * CK:(c + 1) * CK]), _unpack(p_s[r0 // 2:(r0 + CK) // 2, :]),
                     preferred_element_type=f32)
        return pv if acc is None else acc + pv

    def close_sum(l8):
        l = l8.sum(axis=0, keepdims=True)
        bad_s[...] = jnp.where((l >= L_LO) & (l <= L_HI), bad_s[...], 1.0)
        return l

    def fin(h, j, l8, acc):
        ot_s.at[j, h][...] = _pack(acc * (1.0 / close_sum(l8)))

    def body(i, carry):
        zero = jnp.minimum(i, 0)
        never = (lax.broadcasted_iota(jnp.int32, (16, 128), 0) + i) < 0
        lq = [l_s[...]]
        hist = []
        for hh in range(HPB):
            h = i * HPB + hh
            hprev = jnp.maximum(h - 1, 0) if hh == 0 else h - 1
            hnext = jnp.minimum(h + 1, H - 1) if hh == HPB - 1 else h + 1
            kbr, kbase = (kbe_s, (h // 2) * DH) if hh % 2 == 0 else (kbo_s, zero)
            for t in range(NQ):
                slot = t % 2
                l8 = None
                l8v = None
                vacc = None
                for c in range(NC):
                    r0, r1 = BOUNDS[c], BOUNDS[c + 1]
                    s = jnp.dot(_unpack(k_s[h // 8, r0 // 2:r1 // 2, :]), _unpack(ws[slot][...]),
                                preferred_element_type=f32)
                    base = len(hist)
                    hist.extend([s[r:r + 8, 0:128] for r in range(0, r1 - r0, 8)])
                    n_new = len(hist) - base
                    l8 = finish_rows(slot, r0, s, l8)
                    pcs = PIECES[(len(PIECES) * c) // NC:(len(PIECES) * (c + 1)) // NC]
                    for n, (vg, d) in enumerate(pcs):
                        kb = kbr[kbase + d, vg * 16:(vg + 1) * 16, :]
                        ii = base + (n * n_new) // len(pcs) - VOFF
                        if ii >= 0:
                            kb = jnp.where(never, jnp.concatenate([hist[ii]] * 2, axis=0), kb)
                        qb = jnp.concatenate(
                            [jnp.broadcast_to(qf_s.at[slot][d:d + 1, cc * 128:(cc + 1) * 128], (16, 128))
                             for cc in range(TQ // 128)], axis=1)
                        tt = jnp.concatenate([kb] * (TQ // 128), axis=1) * qb
                        vacc = tt if d == 0 else vacc + tt
                        if d == DH - 1:
                            l8v = finish_rows(slot, vg * 16, vacc, l8v)
                    rel, k = divmod(t * NC + c - LAG, NC)
                    hb = hprev if rel < 0 else h
                    acc = pv_chunk(hb, rel % 2, PV_ORDER[k], None if k == 0 else acc_s[...])
                    if k == NC - 1:
                        fin(hb, rel % NQ, lq.pop(0), acc)
                    else:
                        acc_s[...] = acc
                    if c == LAG:
                        if t + 1 < NQ:
                            prep_w(h, t + 1, 1 - slot, hprev if t == 0 else None)
                        else:
                            prep_w(hnext, 0, 1 - slot, h)
                    if hh % 2 == 0:
                        st = t * NC + c
                        for gi in range((len(GENS) * st) // (NQ * NC), (len(GENS) * (st + 1)) // (NQ * NC)):
                            gen_kb(hnext, kbo_s, 0, *GENS[gi], False)
                lq.append(l8 + l8v)
        l_s[...] = lq[0]
        return carry

    lax.fori_loop(0, H // HPB, body, 0)
    close_sum(l_s[...])

    @pl.when(jnp.max(bad_s[...]) > 0.0)
    def _():
        row = lax.broadcasted_iota(jnp.int32, (64, TQ), 0) // 8

        def split(a):
            hi = a.astype(bf16)
            return hi, (a - hi.astype(f32)).astype(bf16)

        def rebuild(b, carry):
            xh, xl = split(_ln(x_s[pl.ds(pl.multiple_of(b * CK, CK), CK), :].astype(f32)))

            def proj(n):
                return (jnp.dot(xh, wqkv_s[n], preferred_element_type=f32)
                        + jnp.dot(xl, wqkv_s[n], preferred_element_type=f32))

            kr = pl.ds(pl.multiple_of(b * (CK // 2), CK // 2), CK // 2)
            for dst, val in zip((k_s, klo_s), split(proj(1))):
                for g in range(4):
                    dst[g, kr, :] = pltpu.bitcast(val[:, g * 128:(g + 1) * 128], u32)
            qc = pl.ds(pl.multiple_of((b % (TQ // CK)) * CK, CK), CK)
            for dst, val in zip((qt_s, qlo_s), split(proj(0) * QSCALE)):
                dst[:, b // (TQ // CK), :, qc] = pltpu.bitcast(val.T, u32).reshape(4, 64, CK)
            return carry

        lax.fori_loop(0, NC, rebuild, 0)

        def unit(u, carry):
            h = u // NQ
            j = u % NQ
            w0_s[...] = jnp.where(row == (h % 8), qt_s[h // 8, j], jnp.uint32(0))
            w1_s[...] = jnp.where(row == (h % 8), qlo_s[h // 8, j], jnp.uint32(0))

            def scores(c, m8):
                kr = pl.ds(pl.multiple_of(c * (CK // 2), CK // 2), CK // 2)
                kh = _unpack(k_s[h // 8, kr, :])
                wh = _unpack(w0_s[...])
                s = (jnp.dot(kh, wh, preferred_element_type=f32)
                     + jnp.dot(_unpack(klo_s[h // 8, kr, :]), wh, preferred_element_type=f32)
                     + jnp.dot(kh, _unpack(w1_s[...]), preferred_element_type=f32))
                s_s[pl.ds(pl.multiple_of(c * CK, CK), CK), :] = s
                return jnp.maximum(m8, s.reshape(CK // 8, 8, TQ).max(axis=0))

            m8 = lax.fori_loop(0, NC, scores, jnp.full((8, TQ), -jnp.inf, f32))
            m = m8.max(axis=0, keepdims=True)

            def probs(c, l8):
                p = jnp.exp2(s_s[pl.ds(pl.multiple_of(c * CK, CK), CK), :] - m)
                p_s[pl.ds(pl.multiple_of(c * (CK // 2), CK // 2), CK // 2), :] = _pack(p)
                return l8 + p.reshape(CK // 8, 8, TQ).sum(axis=0)

            l8 = lax.fori_loop(0, NC, probs, jnp.zeros((8, TQ), f32))
            o = jnp.dot(_unpack(vt_s[h]), _unpack(p_s[0:S // 2, :]), preferred_element_type=f32)
            o = o * (1.0 / l8.sum(axis=0, keepdims=True))
            ot_s[j, h] = _pack(o)
            acc_s[...] = o
            return carry

        lax.fori_loop(0, H * NQ, unit, 0)
        clear_drain()
        l_s[...] = jnp.full((8, TQ), 0.125, f32)

    acc = acc_s[...]
    for k in range(NC - LAG, NC):
        acc = pv_chunk(H - 1, 1, PV_ORDER[k], acc)
    fin(H - 1, NQ - 1, l_s[...], acc)

    w4 = wr_s[0:D].reshape(4, 128).astype(f32)
    wrow = jnp.concatenate([w4[j:j + 1] for j in range(4)], axis=1)
    wr16 = jnp.broadcast_to(wrow, (16, D)).astype(bf16)
    top = []
    topl = []
    nsub = S // EB

    def oproj(n):
        b, lo = divmod(n * EB, TQ)
        o = _unpack(ot_s[b, :, :, lo:lo + EB].reshape(H * 8, EB)).T
        return _mm(o, wo_s)

    def merge(a, b):
        return jnp.maximum(a[0], b[0]), jnp.maximum(jnp.minimum(a[0], b[0]), jnp.maximum(a[1], b[1]))

    def route_key(r, tok):
        bits = pltpu.bitcast(r.astype(bf16).astype(f32), jnp.int32)
        code = ((bits ^ ((bits >> 31) & 0x7FFFFFFF)) >> 16) + 32768
        return pltpu.bitcast(KEY0 + code * S + (S - 1 - tok), f32)

    def push(acc, a, b):
        pair = jnp.maximum(a, b), jnp.minimum(a, b)
        acc[:] = [merge(acc[0], pair)] if acc else [pair]

    def post(n, a):
        r0 = n * EB
        h = x_s[r0:r0 + EB, :].astype(f32) + a
        hn = _ln(h)
        out_s[r0:r0 + EB, :] = (h + hn).astype(bf16)
        hn_s[r0 // 2:(r0 + EB) // 2, :] = _pack(hn)
        if n == nsub - 1:
            r = jnp.sum(hn.astype(bf16).astype(f32) * wrow, axis=1, keepdims=True)
            key = route_key(jnp.broadcast_to(r, (EB, 128)), r0 + lax.broadcasted_iota(jnp.int32, (EB, 128), 0))
            for q in range(0, EB, 16):
                push(top, key[q:q + 8], key[q + 8:q + 16])

    def router(n):
        r0 = n * EB
        r = lax.dot_general(wr16, _unpack(hn_s[r0 // 2:(r0 + EB) // 2, :]), (((1,), (1,)), ((), ())),
                            preferred_element_type=f32)[0:8]
        key = route_key(r, r0 + lax.broadcasted_iota(jnp.int32, (8, EB), 1))
        for q in range(0, EB, 256):
            push(topl, key[:, q:q + 128], key[:, q + 128:q + 256])

    ocps = []

    def send(r0, r1):
        cp = pltpu.make_async_copy(out_s.at[pl.ds(r0, r1 - r0), :], out_hbm.at[pl.ds(r0, r1 - r0), :],
                                   sem_out.at[len(ocps)])
        cp.start()
        ocps.append(cp)
        return r1

    sent = 0
    a_next = oproj(0)
    for n in range(nsub):
        a_cur = a_next
        if n + 1 < nsub:
            a_next = oproj(n + 1)
        if n in OUT_STARTS:
            sent = send(sent, n * EB)
        if n > 0:
            router(n - 1)
        post(n, a_cur)
    send(sent, S)

    best = top[0]
    for sh in (4, 2, 1):
        best = merge(best, (pltpu.roll(best[0], sh, 0), pltpu.roll(best[1], sh, 0)))
    l1 = jnp.max(topl[0][0], axis=1, keepdims=True)
    l2 = jnp.max(jnp.where(topl[0][0] == l1, topl[0][1], topl[0][0]), axis=1, keepdims=True)
    best = merge(best, (jnp.broadcast_to(l1, (8, 128)), jnp.broadcast_to(l2, (8, 128))))
    k1 = pltpu.bitcast(best[0], jnp.int32) - KEY0
    k2 = pltpu.bitcast(best[1], jnp.int32) - KEY0
    i1 = S - 1 - (k1[0, 0] & (S - 1))
    i2 = S - 1 - (k2[0, 0] & (S - 1))

    def gate(k):
        hi = ((k >> 11) - 32768) << 16
        r = pltpu.bitcast((hi ^ ((hi >> 31) & 0x7FFFFFFF)) & -65536, f32)[0:1, 0:1]
        return jax.nn.sigmoid(r)

    t1 = pl.multiple_of((i1 // 16) * 16, 16)
    t2 = pl.multiple_of((i2 // 16) * 16, 16)
    xs = _unpack(jnp.concatenate([hn_s[pl.ds(pl.multiple_of(t // 2, 8), 8), :] for t in (t1, t2)], axis=0))
    g = jnp.dot(xs, wg_s[...], preferred_element_type=f32)
    u = jnp.dot(xs, wu_s[...], preferred_element_type=f32)
    y = jnp.dot((g * jax.nn.sigmoid(g) * u).astype(bf16), wd_s[...], preferred_element_type=f32)
    s1 = gate(k1)
    s2 = gate(k2)
    rows16 = lax.broadcasted_iota(jnp.int32, (16, D), 0)
    for n, t in enumerate((t1, t2)):
        rid = rows16 + t
        yt = y[n * 16:(n + 1) * 16]
        upd = jnp.where(rid == i1, yt * s1, jnp.where(rid == i2, yt * s2, 0.0))
        patch_s[n] = (out_s[pl.ds(t, 16), :].astype(f32) + upd).astype(bf16)
    for cp in ocps:
        cp.wait()
    p1 = pltpu.make_async_copy(patch_s.at[0], out_hbm.at[pl.ds(t1, 16), :], sem_out.at[len(ocps)])
    p2 = pltpu.make_async_copy(patch_s.at[1], out_hbm.at[pl.ds(t2, 16), :], sem_out.at[len(ocps) + 1])
    p1.start()

    @pl.when(t1 != t2)
    def _():
        p2.start()
        p2.wait()

    p1.wait()


@jax.jit
def pallas_sequential_preLN__mha_block__moe_arch_mod__prompt_kernel(
    A_x: jax.Array,
    A_wqkv: jax.Array,
    A_wo: jax.Array,
    B_x: jax.Array,
    B_w_r: jax.Array,
    B_w_gate: jax.Array,
    B_w_up: jax.Array,
    B_w_down: jax.Array,
):
    del B_x
    any_spec = pl.BlockSpec(memory_space=pl.ANY)
    out = pl.pallas_call(
        _kernel,
        out_shape=jax.ShapeDtypeStruct((S, D), bf16),
        in_specs=[any_spec] * 7,
        out_specs=any_spec,
        scratch_shapes=[
            pltpu.VMEM((S, D), bf16),
            pltpu.VMEM((3, D, D), bf16),
            pltpu.VMEM((D, D), bf16),
            pltpu.VMEM((D, F), bf16),
            pltpu.VMEM((D, F), bf16),
            pltpu.VMEM((F, D), bf16),
            pltpu.VMEM((4, S // 2, 128), u32),
            pltpu.VMEM((4, NQ, 64, TQ), u32),
            pltpu.VMEM((H, 8, S), u32),
            pltpu.VMEM((NQ, H, 8, TQ), u32),
            pltpu.VMEM((H, DH, V), f32),
            pltpu.VMEM((H // 2 * DH, V, 128), f32),
            pltpu.VMEM((DH, V, 128), f32),
            pltpu.VMEM((2, DH, TQ), f32),
            pltpu.VMEM((S, TQ), u32),
            pltpu.VMEM((64, TQ), u32),
            pltpu.VMEM((64, TQ), u32),
            pltpu.VMEM((8, TQ), f32),
            pltpu.VMEM((DH, TQ), f32),
            pltpu.VMEM((8, TQ), f32),
            pltpu.VMEM((S // 2, D), u32),
            pltpu.VMEM((S, TQ), f32),
            pltpu.VMEM((4, S // 2, 128), u32),
            pltpu.VMEM((4, NQ, 64, TQ), u32),
            pltpu.VMEM((S, D), bf16),
            pltpu.VMEM((2, 16, D), bf16),
            pltpu.VMEM((4 * D,), bf16),
            pltpu.SemaphoreType.DMA((NQ + 8,)),
            pltpu.SemaphoreType.DMA((len(OUT_STARTS) + 3,)),
        ],
        compiler_params=pltpu.CompilerParams(vmem_limit_bytes=100 * 1024 * 1024),
    )(A_x.reshape(S, D), A_wqkv, A_wo, B_w_r, B_w_gate, B_w_up, B_w_down)
    return out.reshape(1, S, D)
```
